```python
import jax
import jax.numpy as jnp

def _softmax(x, axis=-1):
    return jax.nn.softmax(x, axis=axis)
def _gelu(x):
    return jax.nn.gelu(x, approximate=True)
def _silu(x):
    return jax.nn.silu(x)
def _sigmoid(x):
    return jax.nn.sigmoid(x)
def _layernorm(x, axis=-1, eps=1e-5):
    m = jnp.mean(x, axis=axis, keepdims=True)
    v = jnp.var(x, axis=axis, keepdims=True)
    return (x - m) / jnp.sqrt(v + eps)
def _scatter_add(tgt, idx, src, axis=0):
    return tgt.at[idx].add(src)
def _segment_sum(src, seg, n):
    return jax.ops.segment_sum(src, seg, n)
class _Rng:
    def __init__(self, key):
        self._k = key
    def _next(self):
        self._k, sub = jax.random.split(self._k)
        return sub
    def normal(self, shape):
        return jax.random.normal(self._next(), shape, dtype=jnp.bfloat16)
    def randint(self, lo, hi, shape):
        return jax.random.randint(self._next(), shape, lo, hi, dtype=jnp.int32)
    def uniform(self, shape, lo=0.0, hi=1.0):
        return jax.random.uniform(self._next(), shape, jnp.bfloat16, lo, hi)
    def permutation(self, n):
        return jax.random.permutation(self._next(), n)


kernel_name = 'recurrent_scan__sliding_block_cached__mixer_s_mlp__decode'

def setup_inputs():
    _rng = _Rng(jax.random.key(int.from_bytes(__import__("os").urandom(4), "little")))
    _w = (lambda a: (lambda t: t.astype(jnp.bfloat16) if jnp.issubdtype(t.dtype, jnp.floating) else t)(jnp.asarray(a)))
    def _A_setup():
        B, Sq, D = 1, 1, 512
        Hq, Hkv, Sk, Dh = 32, 32, 32768, 128
        assert Hq % Hkv == 0, (Hq, Hkv)
        return {
            "x": _w((lambda *s: _rng.normal(s) * 0.05)(B, Sq, D)),
            "k_cache": _w((lambda *s: _rng.normal(s) * 0.05)(B, Hkv, Sk, Dh)),
            "v_cache": _w((lambda *s: _rng.normal(s) * 0.05)(B, Hkv, Sk, Dh)),
            "wq": _w((lambda *s: _rng.normal(s) * 0.05)(D, Hq * Dh) * (D ** -0.5)),
            "wo": _w((lambda *s: _rng.normal(s) * 0.05)(Hq * Dh, D) * ((Hq * Dh) ** -0.5)),
        }
    _A_in = _A_setup()

    def _B_setup():
        B, S, D, F = 1, 1, 512, 1376
        return {
            "x":  _w((lambda *s: _rng.normal(s) * 0.05)(B, S, D)),
            "w1": _w((lambda *s: _rng.normal(s) * 0.05)(D, D) * (D ** -0.5)),
            "w2": _w((lambda *s: _rng.normal(s) * 0.05)(D, D) * (D ** -0.5)),
            "w3": _w((lambda *s: _rng.normal(s) * 0.05)(D, F) * (D ** -0.5)),
            "w4": _w((lambda *s: _rng.normal(s) * 0.05)(F, D) * (F ** -0.5)),
        }
    _B_in = _B_setup()

    return {
        "A_x": _A_in["x"],
        "A_k_cache": _A_in["k_cache"],
        "A_v_cache": _A_in["v_cache"],
        "A_wq": _A_in["wq"],
        "A_wo": _A_in["wo"],
        "B_x": _B_in["x"],
        "B_w1": _B_in["w1"],
        "B_w2": _B_in["w2"],
        "B_w3": _B_in["w3"],
        "B_w4": _B_in["w4"],
    }

def reference(A_x, A_k_cache, A_v_cache, A_wq, A_wo, B_x, B_w1, B_w2, B_w3, B_w4):
    def _A_ref(x, k_cache, v_cache, wq, wo):
        B, Sq, D = x.shape
        Hq, Dh = 32, 128
        Hkv, Sk = k_cache.shape[1], k_cache.shape[2]
        W = min(4096, max(256, Sk // 4))
        rep = Hq // Hkv
        q = (lambda x, *d: x.transpose(*d))((x @ wq).reshape(B, Sq, Hq, Dh), 0, 2, 1, 3)
        k = jnp.repeat(k_cache[:, :, Sk - W:, :], rep, axis=1)
        v = jnp.repeat(v_cache[:, :, Sk - W:, :], rep, axis=1)
        scores = jnp.einsum("bhqd,bhkd->bhqk", q, k) * (Dh ** -0.5)
        p = _softmax(scores, axis=-1)
        o = jnp.einsum("bhqk,bhkd->bhqd", p, v)
        return (lambda x, *d: x.transpose(*d))(o, 0, 2, 1, 3).reshape(B, Sq, Hq * Dh) @ wo

    def _B_ref(x, w1, w2, w3, w4):
        B, S, D = x.shape
        h = _gelu(_layernorm(x, axis=-1) @ w1)
        c = D // 4
        g0 = jnp.pad(h[:, :, 0*c:1*c], ((0, 0), (1, 0), (0, 0)))[:, :S, :]
        g1 = jnp.pad(h[:, :, 1*c:2*c], ((0, 0), (0, 1), (0, 0)))[:, 1:, :]
        g2 = jnp.pad(h[:, :, 2*c:3*c], ((0, 0), (2, 0), (0, 0)))[:, :S, :]
        g3 = jnp.pad(h[:, :, 3*c:   ], ((0, 0), (0, 2), (0, 0)))[:, 2:, :]
        hs = jnp.concatenate([g0, g1, g2, g3], axis=-1) @ w2
        x1 = x + hs
        h2 = _gelu(_layernorm(x1, axis=-1) @ w3) @ w4
        return x1 + h2

    x = A_x
    xn = _layernorm(x, axis=-1)
    s = _A_ref(xn, A_k_cache, A_v_cache, A_wq, A_wo)
    g = _silu(_B_ref(xn, B_w1, B_w2, B_w3, B_w4))
    return x + s * g
```

```python
import functools
import jax
import jax.numpy as jnp
import jax.experimental.pallas as pl
import jax.experimental.pallas.tpu as pltpu


def _layernorm(x, eps=1e-5):
    m = jnp.mean(x, axis=-1, keepdims=True)
    xc = x - m
    v = jnp.mean(xc * xc, axis=-1, keepdims=True)
    return xc / jnp.sqrt(v + eps)


class _NoScope:
    def __init__(self, name): pass
    def __enter__(self): return self
    def __exit__(self, *a): return False


def build(L=2, mlp_comp=6, do_compute=True, scopes=False, spread=True, mlp_spread=True, lastprio=1, ring=None):
    scope = jax.named_scope if scopes else _NoScope
    NH, NC, ROWS = 4, 4, 32
    R = ring if ring is not None else (2 if L == 1 else 4)
    assert NC % R == 0 and L < R
    SM, ST = R, R + 1

    def kernel(x_hbm, k_hbm, v_hbm, wq_hbm, wo_hbm, w3_hbm, w4_hbm, o_ref,
               xbuf, kbuf, vbuf, wqbuf, wobuf, w3buf, w4buf, hidbuf, gatebuf, oall, sems):
        H, W, DH = kbuf.shape
        Sk = k_hbm.shape[2]
        D = xbuf.shape[1]
        F = w3buf.shape[0]
        base = Sk - W
        NG = H // NH
        CH = W // NC
        GW = NH * DH
        QA = wq_hbm.shape[0]
        QR = wq_hbm.shape[1]
        HPQ = H // wo_hbm.shape[0]
        f32 = jnp.float32
        bf16 = jnp.bfloat16
        NWQ = QR // 8 // NC
        NWO = DH // 8 // NC
        NM = F // 32

        def k_descs(tg, tc, sem):
            h0 = tg * NH
            out = []
            for i in range(CH // ROWS):
                r = tc * CH + i * ROWS
                def f(r=r):
                    pltpu.make_async_copy(k_hbm.at[0, pl.ds(h0, NH), pl.ds(base + r, ROWS), :],
                                          kbuf.at[pl.ds(h0, NH), pl.ds(r, ROWS), :], sems.at[sem]).start(priority=0)
                out.append(f)
            return out

        def v_descs(tg, tc, sem):
            h0 = tg * NH
            out = []
            for i in range(CH // ROWS):
                r = tc * CH + i * ROWS
                def f(r=r):
                    pltpu.make_async_copy(v_hbm.at[0, pl.ds(h0, NH), pl.ds(base + r, ROWS), :],
                                          vbuf.at[pl.ds(h0, NH), pl.ds(r, ROWS), :], sems.at[sem]).start(priority=1)
                out.append(f)
            return out

        def wq_descs(g, lo, hi, sem, prio=lambda i: 0, cond=None):
            out = []
            for i in range(lo, hi):
                def f(i=i):
                    pltpu.make_async_copy(wq_hbm.at[:, pl.ds(i * 8, 8), pl.ds(pl.multiple_of(g * GW, GW), GW)],
                                          wqbuf.at[g, :, pl.ds(i * 8, 8), :], sems.at[sem]).start(priority=prio(i))
                out.append(f if cond is None else (lambda f=f: pl.when(cond)(f)))
            return out

        def wo_descs(b, lo, hi, sem, prio=lambda i: 1, cond=None):
            out = []
            for i in range(lo, hi):
                def f(i=i):
                    r0 = pl.multiple_of(b * DH + i * 8, 8)
                    pltpu.make_async_copy(wo_hbm.at[:, pl.ds(r0, 8), :], wobuf.at[:, pl.ds(r0, 8), :],
                                          sems.at[sem]).start(priority=prio(i))
                out.append(f if cond is None else (lambda f=f: pl.when(cond)(f)))
            return out

        def mlp_desc(which, n, sem):
            src, dst = ((w3_hbm, w3buf), (w4_hbm, w4buf))[which]
            def f():
                r0 = pl.multiple_of(n * 32, 32)
                pltpu.make_async_copy(src.at[pl.ds(r0, 32), :], dst.at[pl.ds(r0, 32), :], sems.at[sem]).start(priority=which)
            return f

        def interleave(a, b):
            out = []
            for i in range(max(len(a), len(b))):
                if i < len(a): out.append(a[i])
                if i < len(b): out.append(b[i])
            return out

        def spread_in(main, extra, phase):
            if not extra:
                return list(main)
            n = len(main)
            pos = [int((i + phase) * n / len(extra)) for i in range(len(extra))]
            out = []
            e = 0
            for i in range(n + 1):
                while e < len(extra) and pos[e] == i:
                    out.append(extra[e]); e += 1
                if i < n:
                    out.append(main[i])
            return out

        def run(descs):
            for f in descs:
                f()

        def wait(view, sem):
            pltpu.make_async_copy(view, view, sems.at[sem]).wait()

        def kview(g, c): return kbuf.at[pl.ds(g * NH, NH), pl.ds(c * CH, CH), :]
        def vview(g, c): return vbuf.at[pl.ds(g * NH, NH), pl.ds(c * CH, CH), :]
        def wqview(g, p): return wqbuf.at[g, :, pl.ds(p * NWQ * 8, NWQ * 8), :]
        def woview(b, p): return wobuf.at[:, pl.ds(b * DH + p * NWO * 8, NWO * 8), :]

        def wq_target(tg, tc):
            return (tg, NC - 1) if tc == 0 else (tg + 1, tc - 1)

        def batch(tg, tc, has_wq, has_wo, ksem=None, cond_w=None, cond_wq=None, extra0=(), extra1=()):
            sem = tc % R
            ks = k_descs(tg, tc, sem if ksem is None else ksem)
            vs = v_descs(tg, tc, sem)
            a, b = [], []
            if has_wq:
                gq, pq = wq_target(tg, tc)
                a = wq_descs(gq, pq * NWQ, (pq + 1) * NWQ, sem, cond=cond_wq)
            if has_wo:
                b = wo_descs(tg + 1, tc * NWO, (tc + 1) * NWO, sem, cond=cond_w)
            a = a + list(extra0)
            b = b + list(extra1)
            if spread:
                return interleave(spread_in(ks, a, 0.0), spread_in(vs, b, 0.5))
            return interleave(a, b) + interleave(ks, vs)

        with scope('pro'):
            xcp = pltpu.make_async_copy(x_hbm, xbuf, sems.at[SM])
            xcp.start()
            run(wq_descs(0, 0, QR // 8, SM, prio=lambda i: i % 2))
            for t in range(L):
                run(batch(0, t, has_wq=(t > 0), has_wo=True))
        with scope('xwait'):
            xcp.wait()
            wait(wqbuf.at[0], SM)
        x = xbuf[...].astype(f32)
        xn = _layernorm(x).astype(bf16).astype(f32)
        xn8 = jnp.broadcast_to(xn, (8, D)).astype(bf16)
        row = jax.lax.broadcasted_iota(jnp.int32, (8, DH), 0)

        def womm(h, orow, sacc):
            lhs = jnp.broadcast_to(orow, (8, DH)).astype(bf16)
            a, i = h // HPQ, h % HPQ
            return sacc + jnp.dot(lhs, wobuf[a, i * DH:(i + 1) * DH, :], preferred_element_type=f32)

        def group(g, last):
            m = jnp.full((8, 1), -jnp.inf, f32)
            l = jnp.zeros((8, 1), f32)
            acc = jnp.zeros((8, DH), f32)
            sacc = jnp.zeros((8, D), f32)
            qm = None
            for c in range(NC):
                tc = (c + L) % NC
                dg = (c + L) // NC
                tg = g + dg
                with scope('issue'):
                    if last:
                        if dg == 0:
                            final_batch = (tc == NC - 1)
                            run(batch(tg, tc, has_wq=False, has_wo=False, ksem=ST if final_batch else None))
                            if final_batch:
                                run(wo_descs(0, 0, DH // 8, SM, prio=lambda i: lastprio if lastprio < 2 else i % 2))
                    else:
                        e0, e1 = [], []
                        if mlp_spread:
                            s = g * NC + c
                            for k in range(2):
                                n = 2 * s + k
                                e0.append(lambda n=n: pl.when(n < NM)(mlp_desc(0, jnp.minimum(n, NM - 1), SM)))
                                e1.append(lambda n=n: pl.when(n < NM)(mlp_desc(1, jnp.minimum(n, NM - 1), SM)))
                        if dg == 0:
                            run(batch(tg, tc, has_wq=True, has_wo=True, extra0=e0, extra1=e1))
                        else:
                            ok = tg < NG - 1
                            run(batch(tg, tc, has_wq=True, has_wo=True, cond_w=ok, cond_wq=None if tc == 0 else ok,
                                      extra0=e0, extra1=e1))
                        if (not mlp_spread) and c == 0:
                            def allm():
                                for n in range(NM):
                                    mlp_desc(0, n, SM)(); mlp_desc(1, n, SM)()
                            pl.when(g == 1)(allm)
                with scope('wait'):
                    sem = c % R
                    if last and c == NC - 1:
                        wait(kview(g, c), ST)
                    else:
                        wait(kview(g, c), sem)
                        wait(vview(g, c), sem)
                        if last:
                            if c == 0:
                                wait(wqview(g, NC - 1), sem)
                        else:
                            wait(woview(g + 1, c), sem)
                            if c == 0:
                                pl.when(g > 0)(lambda: wait(wqview(g, NC - 1), sem))
                            else:
                                wait(wqview(g + 1, c - 1), sem)
                if c == 0 and do_compute:
                    wqg = wqbuf[g].reshape(D, GW)
                    q = jnp.dot(xn8, wqg, preferred_element_type=f32)
                    qm = [jnp.where(row == j, q[:, j * DH:(j + 1) * DH], 0.0).astype(bf16) for j in range(NH)]
                if do_compute:
                    s = None
                    for j in range(NH):
                        kj = kbuf[g * NH + j, pl.ds(c * CH, CH), :]
                        sj = jax.lax.dot_general(qm[j], kj, (((1,), (1,)), ((), ())), preferred_element_type=f32)
                        s = sj if s is None else s + sj
                    s = s * (DH ** -0.5)
                    m_new = jnp.maximum(m, jnp.max(s, axis=-1, keepdims=True))
                    alpha = jnp.exp(m - m_new)
                    p = jnp.exp(s - m_new)
                    l = l * alpha + jnp.sum(p, axis=-1, keepdims=True)
                    m = m_new
                    pb = p.astype(bf16)
                if last and c < NC - 1 and do_compute:
                    with scope('womm_early'):
                        heads = [h for h in range(H - NH) if h % HPQ != 0]
                        n = len(heads) // (NC - 1)
                        for h in heads[c * n:(c + 1) * n]:
                            sacc = womm(h, oall[h // NH, (h % NH):(h % NH) + 1, :], sacc)
                if last and c == NC - 1:
                    with scope('waitv'):
                        wait(vview(g, c), (c % R))
                if do_compute:
                    pv = jnp.zeros((8, DH), f32)
                    for j in range(NH):
                        vj = vbuf[g * NH + j, pl.ds(c * CH, CH), :]
                        pv = pv + jnp.where(row == j, jnp.dot(pb, vj, preferred_element_type=f32), 0.0)
                    acc = acc * alpha + pv
                if not last:
                    if c == 1:
                        @pl.when(g == mlp_comp)
                        def _():
                            with scope('mlp1'):
                                wait(w3buf, SM)
                                wait(w4buf, SM)
                                y = _layernorm(xn)
                                y8 = jnp.broadcast_to(y, (8, D)).astype(bf16)
                                hid = jax.lax.dot_general(y8, w3buf[...], (((1,), (1,)), ((), ())), preferred_element_type=f32)
                                hidbuf[...] = jax.nn.gelu(hid, approximate=True).astype(bf16)
                    if c == 2:
                        @pl.when(g == mlp_comp)
                        def _():
                            with scope('mlp2'):
                                h2 = jnp.dot(hidbuf[...], w4buf[...], preferred_element_type=f32)
                                b = xn + h2[0:1]
                                gatebuf[...] = b * jax.nn.sigmoid(b)
            o = acc / l if do_compute else acc
            if not last:
                oall[g] = o
                return None
            if do_compute:
                with scope('womm_last'):
                    for j in range(NH):
                        sacc = womm(g * NH + j, o[j:j + 1, :], sacc)
            with scope('waitwo'):
                wait(wobuf.at[:, pl.ds(0, DH), :], SM)
            if do_compute:
                with scope('womm_b0'):
                    for h in range(0, H, HPQ):
                        sacc = womm(h, oall[h // NH, (h % NH):(h % NH) + 1, :], sacc)
            return sacc

        def body(g, _):
            group(g, False)
            return 0
        jax.lax.fori_loop(0, NG - 1, body, 0)
        sacc = group(NG - 1, True)

        with scope('final'):
            o_ref[...] = (x + sacc[0:1, :] * gatebuf[...]).astype(o_ref.dtype)

    def fn(A_x, A_k_cache, A_v_cache, A_wq, A_wo, B_x, B_w1, B_w2, B_w3, B_w4):
        B, Sq, D = A_x.shape
        _, H, Sk, DH = A_k_cache.shape
        W = min(4096, max(256, Sk // 4))
        F = B_w3.shape[1]
        NG = H // NH
        GW = NH * DH
        bf16 = jnp.bfloat16
        anyspec = pl.BlockSpec(memory_space=pl.ANY)
        out = pl.pallas_call(
            kernel,
            in_specs=[anyspec] * 7,
            out_specs=pl.BlockSpec(memory_space=pltpu.VMEM),
            out_shape=jax.ShapeDtypeStruct((1, D), A_x.dtype),
            scratch_shapes=[
                pltpu.VMEM((1, D), bf16),
                pltpu.VMEM((H, W, DH), bf16),
                pltpu.VMEM((H, W, DH), bf16),
                pltpu.VMEM((NG, 4, D // 4, GW), bf16),
                pltpu.VMEM((4, H * DH // 4, D), bf16),
                pltpu.VMEM((F, D), bf16),
                pltpu.VMEM((F, D), bf16),
                pltpu.VMEM((8, F), bf16),
                pltpu.VMEM((1, D), jnp.float32),
                pltpu.VMEM((NG, 8, DH), jnp.float32),
                pltpu.SemaphoreType.DMA((R + 2,)),
            ],
            compiler_params=pltpu.CompilerParams(
                vmem_limit_bytes=100 * 1024 * 1024,
                disable_bounds_checks=True,
            ),
        )(A_x.reshape(1, D), A_k_cache, A_v_cache, A_wq.reshape(4, D // 4, H * DH), A_wo.reshape(4, H * DH // 4, D), B_w3.T, B_w4)
        return out.reshape(B, Sq, D)
    return fn


_impl = build()


@jax.jit
def pallas_recurrent_scan__sliding_block_cached__mixer_s_mlp__decode_kernel(
    A_x: jax.Array,
    A_k_cache: jax.Array,
    A_v_cache: jax.Array,
    A_wq: jax.Array,
    A_wo: jax.Array,
    B_x: jax.Array,
    B_w1: jax.Array,
    B_w2: jax.Array,
    B_w3: jax.Array,
    B_w4: jax.Array,
):
    return _impl(A_x, A_k_cache, A_v_cache, A_wq, A_wo, B_x, B_w1, B_w2, B_w3, B_w4)
```

```python
import jax
import jax.numpy as jnp
import jax.experimental.pallas as pl
import jax.experimental.pallas.tpu as pltpu


def _layernorm(x, eps=1e-5):
    m = jnp.mean(x, axis=-1, keepdims=True)
    xc = x - m
    v = jnp.mean(xc * xc, axis=-1, keepdims=True)
    return xc / jnp.sqrt(v + eps)


class _NoScope:
    def __init__(self, name): pass
    def __enter__(self): return self
    def __exit__(self, *a): return False


def build(mlp_comp=5, do_compute=True, scopes=False, tail='vpu', early_steps=(0,), aprio=1, cprio=1, bounds=False, interpret=False):
    scope = jax.named_scope if scopes else _NoScope
    NH, NC, ROWS, L, R = 4, 4, 32, 2, 4
    MG = 5

    def kernel(x_hbm, k_hbm, v_hbm, wq_hbm, wo_hbm, w3_hbm, w4_hbm, o_ref,
               xbuf, kbuf, vbuf, wqbuf, wobuf, w3buf, w4buf, hidbuf, gatebuf, oall, ocol, sems):
        H, W, DH = kbuf.shape
        Sk = k_hbm.shape[2]
        D = xbuf.shape[1]
        F = w3buf.shape[0]
        base = Sk - W
        NG = H // NH
        CH = W // NC
        GW = NH * DH
        QR = wq_hbm.shape[1]
        NQ = wo_hbm.shape[0]
        HPQ = H // NQ
        f32 = jnp.float32
        bf16 = jnp.bfloat16
        NWQ = QR // 8 // NC
        NWO = DH // 8 // NC
        MR = 32
        MPS = 2
        MPRE = F // MR - MG * NC * MPS

        def copy(src, dst, sem, prio):
            return lambda: pltpu.make_async_copy(src, dst, sems.at[sem]).start(priority=prio)

        def guard(cond, f):
            return f if cond is None else (lambda: pl.when(cond)(f))

        def k_descs(tg, tc, sem):
            return [copy(k_hbm.at[0, pl.ds(tg * NH, NH), pl.ds(base + tc * CH + i * ROWS, ROWS), :],
                         kbuf.at[pl.ds(tg * NH, NH), pl.ds(tc * CH + i * ROWS, ROWS), :], sem, 0)
                    for i in range(CH // ROWS)]

        def v_descs(tg, tc, sem):
            return [copy(v_hbm.at[0, pl.ds(tg * NH, NH), pl.ds(base + tc * CH + i * ROWS, ROWS), :],
                         vbuf.at[pl.ds(tg * NH, NH), pl.ds(tc * CH + i * ROWS, ROWS), :], sem, 1)
                    for i in range(CH // ROWS)]

        def wq_descs(g, lo, hi, sem, prio=lambda i: 0, cond=None):
            col = pl.ds(pl.multiple_of(g * GW, GW), GW)
            return [guard(cond, copy(wq_hbm.at[:, pl.ds(i * 8, 8), col], wqbuf.at[g, :, pl.ds(i * 8, 8), :], sem, prio(i)))
                    for i in range(lo, hi)]

        def wo_descs(b, lo, hi, sem, cond=None):
            out = []
            for i in range(lo, hi):
                rows = pl.ds(pl.multiple_of(b * DH + i * 8, 8), 8)
                out.append(guard(cond, copy(wo_hbm.at[:, rows, :], wobuf.at[:, rows, :], sem, 1)))
            return out

        def mlp_descs(which, lo, n, sem, cond=None):
            src, dst = ((w3_hbm, w3buf), (w4_hbm, w4buf))[which]
            out = []
            for k in range(n):
                rows = pl.ds(pl.multiple_of((lo + k) * MR, MR), MR)
                out.append(guard(cond, copy(src.at[rows, :], dst.at[rows, :], sem, which)))
            return out

        def interleave(a, b):
            out = []
            for i in range(max(len(a), len(b))):
                if i < len(a): out.append(a[i])
                if i < len(b): out.append(b[i])
            return out

        def spread_in(main, extra, phase):
            if not extra:
                return list(main)
            n = len(main)
            pos = [int((i + phase) * n / len(extra)) for i in range(len(extra))]
            out, e = [], 0
            for i in range(n + 1):
                while e < len(extra) and pos[e] == i:
                    out.append(extra[e]); e += 1
                if i < n:
                    out.append(main[i])
            return out

        def run(descs):
            for f in descs:
                f()

        def wait(view, sem):
            pltpu.make_async_copy(view, view, sems.at[sem]).wait()

        def kview(g, c): return kbuf.at[pl.ds(g * NH, NH), pl.ds(c * CH, CH), :]
        def vview(g, c): return vbuf.at[pl.ds(g * NH, NH), pl.ds(c * CH, CH), :]
        def wqview(g, p): return wqbuf.at[g, :, pl.ds(p * NWQ * 8, NWQ * 8), :]
        def woview(b, p): return wobuf.at[:, pl.ds(b * DH + p * NWO * 8, NWO * 8), :]
        def mview(buf, lo, n): return buf.at[pl.ds(lo * MR, n * MR), :]

        def wq_target(tg, tc):
            return (tg, NC - 1) if tc == 0 else (tg + 1, tc - 1)

        def mlp_lo(tg, tc):
            return MPRE + (tg * NC + tc) * MPS

        def batch(tg, tc, wq=True, wo=True, mlp=True, c_wq=None, c_wo=None, c_mlp=None, ksem=None):
            sem = tc
            ks = k_descs(tg, tc, sem if ksem is None else ksem)
            vs = v_descs(tg, tc, sem)
            a, b = [], []
            if wq:
                gq, pq = wq_target(tg, tc)
                if c_wq is not None:
                    gq = jnp.minimum(gq, NG - 1)
                a += wq_descs(gq, pq * NWQ, (pq + 1) * NWQ, sem, cond=c_wq)
            if wo:
                bo = tg + 1 if c_wo is None else jnp.minimum(tg + 1, HPQ - 1)
                b += wo_descs(bo, tc * NWO, (tc + 1) * NWO, sem, cond=c_wo)
            if mlp:
                lo = jnp.minimum(mlp_lo(tg, tc), F // MR - MPS)
                a += mlp_descs(0, lo, MPS, sem, cond=c_mlp)
                b += mlp_descs(1, lo, MPS, sem, cond=c_mlp)
            return interleave(spread_in(ks, a, 0.0), spread_in(vs, b, 0.5))

        PS = 3
        with scope('pro'):
            xcp = pltpu.make_async_copy(x_hbm, xbuf, sems.at[PS])
            xcp.start()
            run(wq_descs(0, 0, QR // 8, PS, prio=lambda i: i % 2))
            run(interleave(mlp_descs(0, 0, MPRE, PS), mlp_descs(1, 0, MPRE, PS)))
            for t in range(L):
                run(batch(0, t, wq=(t > 0)))
        with scope('xwait'):
            xcp.wait()
            wait(wqbuf.at[0], PS)
            wait(mview(w3buf, 0, MPRE), PS)
            wait(mview(w4buf, 0, MPRE), PS)
        x = xbuf[...].astype(f32)
        xn = _layernorm(x).astype(bf16).astype(f32)
        xn8 = jnp.broadcast_to(xn, (8, D)).astype(bf16)
        row = jax.lax.broadcasted_iota(jnp.int32, (8, DH), 0)

        def womm(h, orow, sacc):
            lhs = jnp.broadcast_to(orow, (8, DH)).astype(bf16)
            a, i = h // HPQ, h % HPQ
            return sacc + jnp.dot(lhs, wobuf[a, i * DH:(i + 1) * DH, :], preferred_element_type=f32)

        def orow(h):
            return oall[h // NH, (h % NH):(h % NH) + 1, :]

        def group(g, last):
            m = jnp.full((8, 1), -jnp.inf, f32)
            l = jnp.zeros((8, 1), f32)
            acc = jnp.zeros((8, DH), f32)
            sacc = jnp.zeros((8, D), f32)
            qm = None
            for c in range(NC):
                tc = (c + L) % NC
                dg = (c + L) // NC
                tg = g + dg

                def do_wait():
                    with scope('wait'):
                        if last and c == NC - 1:
                            wait(kview(g, c), 0)
                            return
                        wait(kview(g, c), c)
                        wait(vview(g, c), c)
                        if last:
                            if c == 0:
                                wait(wqview(g, NC - 1), c)
                            return
                        wait(woview(g + 1, c), c)
                        if c == 0:
                            pl.when(g > 0)(lambda: wait(wqview(g, NC - 1), c))
                        else:
                            wait(wqview(g + 1, c - 1), c)

                        @pl.when(g < MG)
                        def _():
                            lo = jnp.minimum(mlp_lo(g, c), F // MR - MPS)
                            wait(mview(w3buf, lo, MPS), c)
                            wait(mview(w4buf, lo, MPS), c)

                if last:
                    if c == 0:
                        with scope('issue'):
                            run(batch(g, tc, wq=False, wo=False, mlp=False))
                        do_wait()
                    elif c == 1:
                        do_wait()
                        with scope('issue'):
                            run(batch(g, tc, wq=False, wo=False, mlp=False, ksem=0))
                            run([copy(wo_hbm.at[pl.ds(1, NQ - 1), pl.ds(i * 8, 8), :],
                                      wobuf.at[pl.ds(1, NQ - 1), pl.ds(i * 8, 8), :], 1, aprio) for i in range(DH // 8)])
                    elif c == 2:
                        do_wait()
                        with scope('issue'):
                            run([copy(wo_hbm.at[0, pl.ds(i * 32, 32), :], wobuf.at[0, pl.ds(i * 32, 32), :], 2, cprio)
                                 for i in range(DH // 32)])
                    else:
                        do_wait()
                else:
                    with scope('issue'):
                        if dg == 0:
                            run(batch(tg, tc, c_mlp=tg < MG))
                        else:
                            ok = tg < NG - 1
                            run(batch(tg, tc, c_wo=ok, c_wq=None if tc == 0 else ok, c_mlp=tg < MG))
                    do_wait()

                if c == 0 and do_compute:
                    wqg = wqbuf[g].reshape(D, GW)
                    q = jnp.dot(xn8, wqg, preferred_element_type=f32)
                    qm = [jnp.where(row == j, q[:, j * DH:(j + 1) * DH], 0.0).astype(bf16) for j in range(NH)]
                if do_compute:
                    s = None
                    for j in range(NH):
                        kj = kbuf[g * NH + j, pl.ds(c * CH, CH), :]
                        sj = jax.lax.dot_general(qm[j], kj, (((1,), (1,)), ((), ())), preferred_element_type=f32)
                        s = sj if s is None else s + sj
                    s = s * (DH ** -0.5)
                    m_new = jnp.maximum(m, jnp.max(s, axis=-1, keepdims=True))
                    alpha = jnp.exp(m - m_new)
                    p = jnp.exp(s - m_new)
                    l = l * alpha + jnp.sum(p, axis=-1, keepdims=True)
                    m = m_new
                    pb = p.astype(bf16)
                if last and c == NC - 1:
                    with scope('waitv'):
                        wait(vview(g, c), c)
                if do_compute:
                    pv = jnp.zeros((8, DH), f32)
                    for j in range(NH):
                        vj = vbuf[g * NH + j, pl.ds(c * CH, CH), :]
                        pv = pv + jnp.where(row == j, jnp.dot(pb, vj, preferred_element_type=f32), 0.0)
                    acc = acc * alpha + pv
                if last and c in early_steps and do_compute:
                    with scope('womm_early'):
                        heads = [h for h in range(H - NH) if h % HPQ != 0]
                        n = len(heads) // len(early_steps)
                        k = early_steps.index(c)
                        for h in heads[k * n:(k + 1) * n]:
                            sacc = womm(h, orow(h), sacc)
                        if tail == 'vpu' and k == 0:
                            ocol[...] = jnp.transpose(jnp.broadcast_to(orow(0), (DH, DH)))
                if not last:
                    if c == 1:
                        @pl.when(g == mlp_comp)
                        def _():
                            with scope('mlp1'):
                                y = _layernorm(xn)
                                y8 = jnp.broadcast_to(y, (8, D)).astype(bf16)
                                hid = jax.lax.dot_general(y8, w3buf[...], (((1,), (1,)), ((), ())), preferred_element_type=f32)
                                hidbuf[...] = jax.nn.gelu(hid, approximate=True).astype(bf16)
                    if c == 2:
                        @pl.when(g == mlp_comp)
                        def _():
                            with scope('mlp2'):
                                h2 = jnp.dot(hidbuf[...], w4buf[...], preferred_element_type=f32)
                                b = xn + h2[0:1]
                                gatebuf[...] = b * jax.nn.sigmoid(b)
            o = acc / l if do_compute else acc
            if not last:
                oall[g] = o
                return None
            if do_compute:
                with scope('womm_last'):
                    for j in range(NH):
                        sacc = womm(g * NH + j, o[j:j + 1, :], sacc)
            with scope('waitA'):
                wait(wobuf.at[pl.ds(1, NQ - 1), pl.ds(0, DH), :], 1)
            if do_compute:
                with scope('wommA'):
                    for h in range(HPQ, H, HPQ):
                        sacc = womm(h, orow(h), sacc)
            s_row = sacc[0:1, :]
            gate = gatebuf[...]
            with scope('waitC'):
                wait(wobuf.at[0, pl.ds(0, DH), :], 2)
            if do_compute:
                with scope('wommC'):
                    if tail == 'mxu':
                        s_row = s_row + womm(0, orow(0), jnp.zeros((8, D), f32))[0:1, :]
                    else:
                        w0 = wobuf[0, 0:DH, :].astype(f32)
                        oc = ocol[...]
                        parts = []
                        for n in range(D // DH):
                            pr = w0[:, n * DH:(n + 1) * DH] * oc
                            parts.append(jnp.sum(pr, axis=0, keepdims=True))
                        s_row = s_row + jnp.concatenate(parts, axis=1)
            with scope('final'):
                o_ref[...] = (x + s_row * gate).astype(o_ref.dtype)
            return None

        def body(g, _):
            group(g, False)
            return 0
        jax.lax.fori_loop(0, NG - 1, body, 0)
        group(NG - 1, True)

    def fn(A_x, A_k_cache, A_v_cache, A_wq, A_wo, B_x, B_w1, B_w2, B_w3, B_w4):
        B, Sq, D = A_x.shape
        _, H, Sk, DH = A_k_cache.shape
        W = min(4096, max(256, Sk // 4))
        F = B_w3.shape[1]
        NG = H // NH
        GW = NH * DH
        bf16 = jnp.bfloat16
        anyspec = pl.BlockSpec(memory_space=pl.ANY)
        out = pl.pallas_call(
            kernel,
            in_specs=[anyspec] * 7,
            out_specs=pl.BlockSpec(memory_space=pltpu.VMEM),
            out_shape=jax.ShapeDtypeStruct((1, D), A_x.dtype),
            scratch_shapes=[
                pltpu.VMEM((1, D), bf16),
                pltpu.VMEM((H, W, DH), bf16),
                pltpu.VMEM((H, W, DH), bf16),
                pltpu.VMEM((NG, 4, D // 4, GW), bf16),
                pltpu.VMEM((4, H * DH // 4, D), bf16),
                pltpu.VMEM((F, D), bf16),
                pltpu.VMEM((F, D), bf16),
                pltpu.VMEM((8, F), bf16),
                pltpu.VMEM((1, D), jnp.float32),
                pltpu.VMEM((NG, 8, DH), jnp.float32),
                pltpu.VMEM((DH, DH), jnp.float32),
                pltpu.SemaphoreType.DMA((R,)),
            ],
            compiler_params=pltpu.CompilerParams(
                vmem_limit_bytes=100 * 1024 * 1024,
                disable_bounds_checks=not bounds,
            ),
            interpret=interpret,
        )(A_x.reshape(1, D), A_k_cache, A_v_cache, A_wq.reshape(4, D // 4, H * DH), A_wo.reshape(4, H * DH // 4, D), B_w3.T, B_w4)
        return out.reshape(B, Sq, D)
    return fn


_impl = build()


@jax.jit
def pallas_recurrent_scan__sliding_block_cached__mixer_s_mlp__decode_kernel(
    A_x: jax.Array,
    A_k_cache: jax.Array,
    A_v_cache: jax.Array,
    A_wq: jax.Array,
    A_wo: jax.Array,
    B_x: jax.Array,
    B_w1: jax.Array,
    B_w2: jax.Array,
    B_w3: jax.Array,
    B_w4: jax.Array,
):
    return _impl(A_x, A_k_cache, A_v_cache, A_wq, A_wo, B_x, B_w1, B_w2, B_w3, B_w4)
```

```python
import jax
import jax.numpy as jnp
import jax.experimental.pallas as pl
import jax.experimental.pallas.tpu as pltpu


def _layernorm(x, eps=1e-5):
    m = jnp.mean(x, axis=-1, keepdims=True)
    xc = x - m
    v = jnp.mean(xc * xc, axis=-1, keepdims=True)
    return xc / jnp.sqrt(v + eps)


class _NoScope:
    def __init__(self, name): pass
    def __enter__(self): return self
    def __exit__(self, *a): return False


def build(mlp_comp=5, do_compute=True, scopes=False, tail='vpu', early_steps=(0,), aprio=1, cprio=1, bounds=False, interpret=False, mlp_aligned=True, pro_spread=True, ROWS=24, ROWS_LAST=None, last_from=2, ph0=0.5, ph1=0.5, MR=32, wq_split=1, wo_rows=8, QA=4, pph=None, moff=5, mpos=None, vrev=False, krev=False, swap_w=False, swap_m=False, swap_kv=False):
    scope = jax.named_scope if scopes else _NoScope
    NH, NC, L, R = 4, 4, 2, 4
    RL = ROWS if ROWS_LAST is None else ROWS_LAST
    MG = 5

    def kernel(x_hbm, k_hbm, v_hbm, wq_hbm, wo_hbm, w3_hbm, w4_hbm, o_ref,
               xbuf, kbuf, vbuf, wqbuf, wobuf, w3buf, w4buf, hidbuf, gatebuf, oall, ocol, sems):
        H, W, DH = kbuf.shape
        Sk = k_hbm.shape[2]
        D = xbuf.shape[1]
        F = w3buf.shape[0]
        base = Sk - W
        NG = H // NH
        CH = W // NC
        GW = NH * DH
        QR = wq_hbm.shape[1]
        NQ = wo_hbm.shape[0]
        HPQ = H // NQ
        f32 = jnp.float32
        bf16 = jnp.bfloat16
        NWQ = QR // 8 // NC
        NWO = DH // 8 // NC
        MPS = 64 // MR
        MPRE = F // MR - MG * NC * MPS

        def copy(src, dst, sem, prio):
            return lambda: pltpu.make_async_copy(src, dst, sems.at[sem]).start(priority=prio)

        def guard(cond, f):
            return f if cond is None else (lambda: pl.when(cond)(f))

        rb = [min(-(-CH * c // ROWS) * ROWS, W) for c in range(NC + 1)]

        def pieces(c, rows):
            return [(r, min(rows, rb[c + 1] - r)) for r in range(rb[c], rb[c + 1], rows)]

        def k_descs(tg, tc, sem, rows, prio=0):
            return [copy(k_hbm.at[0, pl.ds(tg * NH, NH), pl.ds(base + r, n), :],
                         kbuf.at[pl.ds(tg * NH, NH), pl.ds(r, n), :], sem, prio) for r, n in pieces(tc, rows)]

        def v_descs(tg, tc, sem, rows, prio=1):
            return [copy(v_hbm.at[0, pl.ds(tg * NH, NH), pl.ds(base + r, n), :],
                         vbuf.at[pl.ds(tg * NH, NH), pl.ds(r, n), :], sem, prio) for r, n in pieces(tc, rows)]

        def wq_descs(g, lo, hi, sem, prio=lambda i: 0, cond=None):
            cw = GW // wq_split
            return [guard(cond, copy(wq_hbm.at[:, pl.ds(i * 8, 8), pl.ds(pl.multiple_of(g * GW + k * cw, cw), cw)],
                                     wqbuf.at[g, :, pl.ds(i * 8, 8), pl.ds(k * cw, cw)], sem, prio(i)))
                    for i in range(lo, hi) for k in range(wq_split)]

        def wo_descs(b, lo, hi, sem, cond=None, prio=1):
            out = []
            for i in range(lo * 8 // wo_rows, hi * 8 // wo_rows):
                rows = pl.ds(pl.multiple_of(b * DH + i * wo_rows, 8), wo_rows)
                out.append(guard(cond, copy(wo_hbm.at[:, rows, :], wobuf.at[:, rows, :], sem, prio)))
            return out

        def mlp_descs(which, lo, n, sem, cond=None, prio=None):
            src, dst = ((w3_hbm, w3buf), (w4_hbm, w4buf))[which]
            out = []
            for k in range(n):
                rows = pl.ds(pl.multiple_of((lo + k) * MR, MR), MR)
                out.append(guard(cond, copy(src.at[rows, :], dst.at[rows, :], sem, which if prio is None else prio)))
            return out

        def interleave(a, b):
            out = []
            for i in range(max(len(a), len(b))):
                if i < len(a): out.append(a[i])
                if i < len(b): out.append(b[i])
            return out

        def spread_in(main, extra, phase):
            if not extra:
                return list(main)
            n = len(main)
            pos = [int((i + phase) * n / len(extra)) for i in range(len(extra))]
            out, e = [], 0
            for i in range(n + 1):
                while e < len(extra) and pos[e] == i:
                    out.append(extra[e]); e += 1
                if i < n:
                    out.append(main[i])
            return out

        def run(descs):
            for f in descs:
                f()

        def wait(view, sem):
            pltpu.make_async_copy(view, view, sems.at[sem]).wait()

        def kview(g, c): return kbuf.at[pl.ds(g * NH, NH), pl.ds(rb[c], rb[c + 1] - rb[c]), :]
        def vview(g, c): return vbuf.at[pl.ds(g * NH, NH), pl.ds(rb[c], rb[c + 1] - rb[c]), :]
        def wqview(g, p): return wqbuf.at[g, :, pl.ds(p * NWQ * 8, NWQ * 8), :]
        def woview(b, p): return wobuf.at[:, pl.ds(b * DH + p * NWO * 8, NWO * 8), :]
        def mview(buf, lo, n): return buf.at[pl.ds(lo * MR, n * MR), :]

        def wq_target(tg, tc):
            return (tg, NC - 1) if tc == 0 else (tg + 1, tc - 1)

        def mlp_lo(tg, tc):
            return MPRE + (tg * NC + tc) * MPS

        def batch(tg, tc, wq=True, wo=True, mlp=True, c_wq=None, c_wo=None, c_mlp=None, ksem=None, extra0=(), extra1=(), rows=ROWS, phs=None):
            sem = tc
            steady = ksem is None
            ks = k_descs(tg, tc, sem if ksem is None else ksem, rows)
            vs = v_descs(tg, tc, sem, rows)
            if vrev: vs = vs[::-1]
            if krev: ks = ks[::-1]
            if swap_kv and steady:
                ks, vs = v_descs(tg, tc, sem, rows, 0), k_descs(tg, tc, sem, rows, 1)
            a, b = [], []
            if wq:
                gq, pq = wq_target(tg, tc)
                if c_wq is not None:
                    gq = jnp.minimum(gq, NG - 1)
                wql = wq_descs(gq, pq * NWQ, (pq + 1) * NWQ, sem, prio=lambda i: 1 if swap_w else 0, cond=c_wq)
                if swap_w: b += wql
                else: a += wql
            if wo:
                bo = tg + 1 if c_wo is None else jnp.minimum(tg + 1, HPQ - 1)
                wol = wo_descs(bo, tc * NWO, (tc + 1) * NWO, sem, cond=c_wo, prio=0 if swap_w else 1)
                if swap_w: a += wol
                else: b += wol
            a += list(extra0)
            b += list(extra1)
            if mlp and not mlp_aligned:
                lo = jnp.minimum(mlp_lo(tg, tc), F // MR - MPS)
                a += mlp_descs(0, lo, MPS, sem, cond=c_mlp)
                b += mlp_descs(1, lo, MPS, sem, cond=c_mlp)
            f0, f1 = (ph0, ph1) if phs is None else phs
            p0, p1 = spread_in(ks, a, f0), spread_in(vs, b, f1)
            if mlp and mlp_aligned:
                lo = jnp.minimum(mlp_lo(tg, tc), F // MR - MPS)
                m3, m4 = mlp_descs(0, lo, MPS, sem, cond=c_mlp), mlp_descs(1, lo, MPS, sem, cond=c_mlp)
                if swap_m:
                    m3, m4 = mlp_descs(1, lo, MPS, sem, cond=c_mlp, prio=0), mlp_descs(0, lo, MPS, sem, cond=c_mlp, prio=1)
                n = min(len(p0), len(p1))
                for k in range(MPS - 1, -1, -1):
                    pos = (2 * k + 1) * n // (2 * MPS) + moff if mpos is None else int(mpos[k] * n)
                    p0.insert(pos, m3[k]); p1.insert(pos, m4[k])
            return interleave(p0, p1)

        PS = 3
        with scope('pro'):
            xcp = pltpu.make_async_copy(x_hbm, xbuf, sems.at[PS])
            xcp.start()
            if pro_spread:
                nq = QR // 8
                nwo = NWO * 8 // wo_rows
                n0 = min(nq, (nq * wq_split + nwo + 1) // 2 // wq_split)
                e0 = wq_descs(0, 0, n0, PS, prio=lambda i: 0) + mlp_descs(0, 0, MPRE, PS)
                e1 = wq_descs(0, n0, nq, PS, prio=lambda i: 1) + mlp_descs(1, 0, MPRE, PS)
                run(batch(0, 0, wq=False, extra0=e0, extra1=e1, phs=None if pph is None else (pph, pph)))
                run(batch(0, 1))
            else:
                run(wq_descs(0, 0, QR // 8, PS, prio=lambda i: i % 2))
                run(interleave(mlp_descs(0, 0, MPRE, PS), mlp_descs(1, 0, MPRE, PS)))
                for t in range(L):
                    run(batch(0, t, wq=(t > 0)))
        with scope('xwait'):
            xcp.wait()
            wait(wqbuf.at[0], PS)
            wait(mview(w3buf, 0, MPRE), PS)
            wait(mview(w4buf, 0, MPRE), PS)
        x = xbuf[...].astype(f32)
        xn = _layernorm(x).astype(bf16).astype(f32)
        xn8 = jnp.broadcast_to(xn, (8, D)).astype(bf16)
        row = jax.lax.broadcasted_iota(jnp.int32, (8, DH), 0)

        def womm(h, orow, sacc):
            lhs = jnp.broadcast_to(orow, (8, DH)).astype(bf16)
            a, i = h // HPQ, h % HPQ
            return sacc + jnp.dot(lhs, wobuf[a, i * DH:(i + 1) * DH, :], preferred_element_type=f32)

        def orow(h):
            return oall[h // NH, (h % NH):(h % NH) + 1, :]

        def group(g, last):
            m = jnp.full((8, 1), -jnp.inf, f32)
            l = jnp.zeros((8, 1), f32)
            acc = jnp.zeros((8, DH), f32)
            sacc = jnp.zeros((8, D), f32)
            qm = None
            for c in range(NC):
                tc = (c + L) % NC
                dg = (c + L) // NC
                tg = g + dg

                def do_wait():
                    with scope('wait'):
                        if last and c == NC - 1:
                            wait(kview(g, c), 0)
                            return
                        wait(kview(g, c), c)
                        wait(vview(g, c), c)
                        if last:
                            if c == 0:
                                wait(wqview(g, NC - 1), c)
                            return
                        wait(woview(g + 1, c), c)
                        if c == 0:
                            pl.when(g > 0)(lambda: wait(wqview(g, NC - 1), c))
                        else:
                            wait(wqview(g + 1, c - 1), c)

                        @pl.when(g < MG)
                        def _():
                            lo = jnp.minimum(mlp_lo(g, c), F // MR - MPS)
                            wait(mview(w3buf, lo, MPS), c)
                            wait(mview(w4buf, lo, MPS), c)

                if last:
                    if c == 0:
                        with scope('issue'):
                            run(batch(g, tc, wq=False, wo=False, mlp=False, rows=RL if last_from <= 2 else ROWS))
                        do_wait()
                    elif c == 1:
                        do_wait()
                        with scope('issue'):
                            run(batch(g, tc, wq=False, wo=False, mlp=False, ksem=0, rows=RL))
                            run([copy(wo_hbm.at[pl.ds(1, NQ - 1), pl.ds(i * 8, 8), :],
                                      wobuf.at[pl.ds(1, NQ - 1), pl.ds(i * 8, 8), :], 1, aprio) for i in range(DH // 8)])
                    elif c == 2:
                        do_wait()
                        with scope('issue'):
                            run([copy(wo_hbm.at[0, pl.ds(i * 32, 32), :], wobuf.at[0, pl.ds(i * 32, 32), :], 2, cprio)
                                 for i in range(DH // 32)])
                    else:
                        do_wait()
                else:
                    with scope('issue'):
                        if dg == 0:
                            run(batch(tg, tc, c_mlp=tg < MG))
                        else:
                            ok = tg < NG - 1
                            run(batch(tg, tc, c_wo=ok, c_wq=None if tc == 0 else ok, c_mlp=tg < MG))
                    do_wait()

                if c == 0 and do_compute:
                    wqg = wqbuf[g].reshape(D, GW)
                    q = jnp.dot(xn8, wqg, preferred_element_type=f32)
                    qm = [jnp.where(row == j, q[:, j * DH:(j + 1) * DH], 0.0).astype(bf16) for j in range(NH)]
                if do_compute:
                    s = None
                    for j in range(NH):
                        kj = kbuf[g * NH + j, pl.ds(c * CH, CH), :]
                        sj = jax.lax.dot_general(qm[j], kj, (((1,), (1,)), ((), ())), preferred_element_type=f32)
                        s = sj if s is None else s + sj
                    s = s * (DH ** -0.5)
                    m_new = jnp.maximum(m, jnp.max(s, axis=-1, keepdims=True))
                    alpha = jnp.exp(m - m_new)
                    p = jnp.exp(s - m_new)
                    l = l * alpha + jnp.sum(p, axis=-1, keepdims=True)
                    m = m_new
                    pb = p.astype(bf16)
                if last and c == NC - 1:
                    with scope('waitv'):
                        wait(vview(g, c), c)
                if do_compute:
                    pv = jnp.zeros((8, DH), f32)
                    for j in range(NH):
                        vj = vbuf[g * NH + j, pl.ds(c * CH, CH), :]
                        pv = pv + jnp.where(row == j, jnp.dot(pb, vj, preferred_element_type=f32), 0.0)
                    acc = acc * alpha + pv
                if last and c in early_steps and do_compute:
                    with scope('womm_early'):
                        heads = [h for h in range(H - NH) if h % HPQ != 0]
                        n = len(heads) // len(early_steps)
                        k = early_steps.index(c)
                        for h in heads[k * n:(k + 1) * n]:
                            sacc = womm(h, orow(h), sacc)
                        if tail == 'vpu' and k == 0:
                            ocol[...] = jnp.transpose(jnp.broadcast_to(orow(0), (DH, DH)))
                if not last:
                    if c == 1:
                        @pl.when(g == mlp_comp)
                        def _():
                            with scope('mlp1'):
                                y = _layernorm(xn)
                                y8 = jnp.broadcast_to(y, (8, D)).astype(bf16)
                                hid = jax.lax.dot_general(y8, w3buf[...], (((1,), (1,)), ((), ())), preferred_element_type=f32)
                                hidbuf[...] = jax.nn.gelu(hid, approximate=True).astype(bf16)
                    if c == 2:
                        @pl.when(g == mlp_comp)
                        def _():
                            with scope('mlp2'):
                                h2 = jnp.dot(hidbuf[...], w4buf[...], preferred_element_type=f32)
                                b = xn + h2[0:1]
                                gatebuf[...] = b * jax.nn.sigmoid(b)
            o = acc / l if do_compute else acc
            if not last:
                oall[g] = o
                return None
            if do_compute:
                with scope('womm_last'):
                    for j in range(NH):
                        sacc = womm(g * NH + j, o[j:j + 1, :], sacc)
            with scope('waitA'):
                wait(wobuf.at[pl.ds(1, NQ - 1), pl.ds(0, DH), :], 1)
            if do_compute:
                with scope('wommA'):
                    for h in range(HPQ, H, HPQ):
                        sacc = womm(h, orow(h), sacc)
            s_row = sacc[0:1, :]
            gate = gatebuf[...]
            with scope('waitC'):
                wait(wobuf.at[0, pl.ds(0, DH), :], 2)
            if do_compute:
                with scope('wommC'):
                    if tail == 'mxu':
                        s_row = s_row + womm(0, orow(0), jnp.zeros((8, D), f32))[0:1, :]
                    else:
                        w0 = wobuf[0, 0:DH, :].astype(f32)
                        oc = ocol[...]
                        parts = []
                        for n in range(D // DH):
                            pr = w0[:, n * DH:(n + 1) * DH] * oc
                            parts.append(jnp.sum(pr, axis=0, keepdims=True))
                        s_row = s_row + jnp.concatenate(parts, axis=1)
            with scope('final'):
                o_ref[...] = (x + s_row * gate).astype(o_ref.dtype)
            return None

        def body(g, _):
            group(g, False)
            return 0
        jax.lax.fori_loop(0, NG - 1, body, 0)
        group(NG - 1, True)

    def fn(A_x, A_k_cache, A_v_cache, A_wq, A_wo, B_x, B_w1, B_w2, B_w3, B_w4):
        B, Sq, D = A_x.shape
        _, H, Sk, DH = A_k_cache.shape
        W = min(4096, max(256, Sk // 4))
        F = B_w3.shape[1]
        NG = H // NH
        GW = NH * DH
        bf16 = jnp.bfloat16
        anyspec = pl.BlockSpec(memory_space=pl.ANY)
        out = pl.pallas_call(
            kernel,
            in_specs=[anyspec] * 7,
            out_specs=pl.BlockSpec(memory_space=pltpu.VMEM),
            out_shape=jax.ShapeDtypeStruct((1, D), A_x.dtype),
            scratch_shapes=[
                pltpu.VMEM((1, D), bf16),
                pltpu.VMEM((H, W, DH), bf16),
                pltpu.VMEM((H, W, DH), bf16),
                pltpu.VMEM((NG, QA, D // QA, GW), bf16),
                pltpu.VMEM((4, H * DH // 4, D), bf16),
                pltpu.VMEM((F, D), bf16),
                pltpu.VMEM((F, D), bf16),
                pltpu.VMEM((8, F), bf16),
                pltpu.VMEM((1, D), jnp.float32),
                pltpu.VMEM((NG, 8, DH), jnp.float32),
                pltpu.VMEM((DH, DH), jnp.float32),
                pltpu.SemaphoreType.DMA((R,)),
            ],
            compiler_params=pltpu.CompilerParams(
                vmem_limit_bytes=100 * 1024 * 1024,
                disable_bounds_checks=not bounds,
            ),
            interpret=interpret,
        )(A_x.reshape(1, D), A_k_cache, A_v_cache, A_wq.reshape(QA, D // QA, H * DH), A_wo.reshape(4, H * DH // 4, D), B_w3.T, B_w4)
        return out.reshape(B, Sq, D)
    return fn


_impl = build()


@jax.jit
def pallas_recurrent_scan__sliding_block_cached__mixer_s_mlp__decode_kernel(
    A_x: jax.Array,
    A_k_cache: jax.Array,
    A_v_cache: jax.Array,
    A_wq: jax.Array,
    A_wo: jax.Array,
    B_x: jax.Array,
    B_w1: jax.Array,
    B_w2: jax.Array,
    B_w3: jax.Array,
    B_w4: jax.Array,
):
    return _impl(A_x, A_k_cache, A_v_cache, A_wq, A_wo, B_x, B_w1, B_w2, B_w3, B_w4)
```

```python
import jax
import jax.numpy as jnp
import jax.experimental.pallas as pl
import jax.experimental.pallas.tpu as pltpu


def _layernorm(x, eps=1e-5):
    m = jnp.mean(x, axis=-1, keepdims=True)
    xc = x - m
    v = jnp.mean(xc * xc, axis=-1, keepdims=True)
    return xc / jnp.sqrt(v + eps)


class _NoScope:
    def __init__(self, name): pass
    def __enter__(self): return self
    def __exit__(self, *a): return False


def build(mlp_comp=5, do_compute=True, scopes=False, tail='vpu', early_steps=(0,), aprio=1, cprio=1, bounds=False, interpret=False, mlp_aligned=True, pro_spread=True, ROWS=24, ROWS_LAST=None, last_from=2, ph0=0.5, ph1=0.5, MR=32, wq_split=1, wo_rows=8, QA=4, pph=None, moff=5, mpos=None, vrev=False, krev=False, swap_w=False, swap_m=False, swap_kv=False, x1rows=16, R3=96):
    scope = jax.named_scope if scopes else _NoScope
    NH, NC, L, R = 4, 4, 2, 4
    RL = ROWS if ROWS_LAST is None else ROWS_LAST
    MG = 5

    def kernel(x_hbm, k_hbm, v_hbm, wq_hbm, wo_hbm, w3_hbm, w4_hbm, o_ref,
               xbuf, kbuf, vbuf, wqbuf, wobuf, w3buf, w4buf, hidbuf, gatebuf, oall, ocol, sems):
        H, W, DH = kbuf.shape
        Sk = k_hbm.shape[2]
        D = xbuf.shape[1]
        F = w3buf.shape[0]
        base = Sk - W
        NG = H // NH
        CH = W // NC
        GW = NH * DH
        QR = wq_hbm.shape[1]
        NQ = wo_hbm.shape[0]
        HPQ = H // NQ
        f32 = jnp.float32
        bf16 = jnp.bfloat16
        NWQ = QR // 8 // NC
        NWO = DH // 8 // NC
        MPS = 64 // MR
        MPRE = F // MR - MG * NC * MPS

        def copy(src, dst, sem, prio):
            return lambda: pltpu.make_async_copy(src, dst, sems.at[sem]).start(priority=prio)

        def guard(cond, f):
            return f if cond is None else (lambda: pl.when(cond)(f))

        rb = [min(-(-CH * c // ROWS) * ROWS, W) for c in range(NC + 1)]

        def pieces(c, rows):
            return [(r, min(rows, rb[c + 1] - r)) for r in range(rb[c], rb[c + 1], rows)]

        def k_descs(tg, tc, sem, rows, prio=0):
            return [copy(k_hbm.at[0, pl.ds(tg * NH, NH), pl.ds(base + r, n), :],
                         kbuf.at[pl.ds(tg * NH, NH), pl.ds(r, n), :], sem, prio) for r, n in pieces(tc, rows)]

        def v_descs(tg, tc, sem, rows, prio=1):
            return [copy(v_hbm.at[0, pl.ds(tg * NH, NH), pl.ds(base + r, n), :],
                         vbuf.at[pl.ds(tg * NH, NH), pl.ds(r, n), :], sem, prio) for r, n in pieces(tc, rows)]

        def wq_descs(g, lo, hi, sem, prio=lambda i: 0, cond=None):
            cw = GW // wq_split
            return [guard(cond, copy(wq_hbm.at[:, pl.ds(i * 8, 8), pl.ds(pl.multiple_of(g * GW + k * cw, cw), cw)],
                                     wqbuf.at[g, :, pl.ds(i * 8, 8), pl.ds(k * cw, cw)], sem, prio(i)))
                    for i in range(lo, hi) for k in range(wq_split)]

        def wo_descs(b, lo, hi, sem, cond=None, prio=1):
            out = []
            for i in range(lo * 8 // wo_rows, hi * 8 // wo_rows):
                rows = pl.ds(pl.multiple_of(b * DH + i * wo_rows, 8), wo_rows)
                out.append(guard(cond, copy(wo_hbm.at[:, rows, :], wobuf.at[:, rows, :], sem, prio)))
            return out

        def mlp_descs(which, lo, n, sem, cond=None, prio=None):
            src, dst = ((w3_hbm, w3buf), (w4_hbm, w4buf))[which]
            out = []
            for k in range(n):
                rows = pl.ds(pl.multiple_of((lo + k) * MR, MR), MR)
                out.append(guard(cond, copy(src.at[rows, :], dst.at[rows, :], sem, which if prio is None else prio)))
            return out

        def interleave(a, b):
            out = []
            for i in range(max(len(a), len(b))):
                if i < len(a): out.append(a[i])
                if i < len(b): out.append(b[i])
            return out

        def spread_in(main, extra, phase):
            if not extra:
                return list(main)
            n = len(main)
            pos = [int((i + phase) * n / len(extra)) for i in range(len(extra))]
            out, e = [], 0
            for i in range(n + 1):
                while e < len(extra) and pos[e] == i:
                    out.append(extra[e]); e += 1
                if i < n:
                    out.append(main[i])
            return out

        def run(descs):
            for f in descs:
                f()

        def wait(view, sem):
            pltpu.make_async_copy(view, view, sems.at[sem]).wait()

        def kview(g, c): return kbuf.at[pl.ds(g * NH, NH), pl.ds(rb[c], rb[c + 1] - rb[c]), :]
        def vview(g, c): return vbuf.at[pl.ds(g * NH, NH), pl.ds(rb[c], rb[c + 1] - rb[c]), :]
        def wqview(g, p): return wqbuf.at[g, :, pl.ds(p * NWQ * 8, NWQ * 8), :]
        def woview(b, p): return wobuf.at[:, pl.ds(b * DH + p * NWO * 8, NWO * 8), :]
        def mview(buf, lo, n): return buf.at[pl.ds(lo * MR, n * MR), :]

        def wq_target(tg, tc):
            return (tg, NC - 1) if tc == 0 else (tg + 1, tc - 1)

        def mlp_lo(tg, tc):
            return MPRE + (tg * NC + tc) * MPS

        def batch(tg, tc, wq=True, wo=True, mlp=True, c_wq=None, c_wo=None, c_mlp=None, ksem=None, extra0=(), extra1=(), rows=ROWS, phs=None):
            sem = tc
            steady = ksem is None
            ks = k_descs(tg, tc, sem if ksem is None else ksem, rows)
            vs = v_descs(tg, tc, sem, rows)
            if vrev: vs = vs[::-1]
            if krev: ks = ks[::-1]
            if swap_kv and steady:
                ks, vs = v_descs(tg, tc, sem, rows, 0), k_descs(tg, tc, sem, rows, 1)
            a, b = [], []
            if wq:
                gq, pq = wq_target(tg, tc)
                if c_wq is not None:
                    gq = jnp.minimum(gq, NG - 1)
                wql = wq_descs(gq, pq * NWQ, (pq + 1) * NWQ, sem, prio=lambda i: 1 if swap_w else 0, cond=c_wq)
                if swap_w: b += wql
                else: a += wql
            if wo:
                bo = tg + 1 if c_wo is None else jnp.minimum(tg + 1, HPQ - 1)
                wol = wo_descs(bo, tc * NWO, (tc + 1) * NWO, sem, cond=c_wo, prio=0 if swap_w else 1)
                if swap_w: a += wol
                else: b += wol
            a += list(extra0)
            b += list(extra1)
            if mlp and not mlp_aligned:
                lo = jnp.minimum(mlp_lo(tg, tc), F // MR - MPS)
                a += mlp_descs(0, lo, MPS, sem, cond=c_mlp)
                b += mlp_descs(1, lo, MPS, sem, cond=c_mlp)
            f0, f1 = (ph0, ph1) if phs is None else phs
            p0, p1 = spread_in(ks, a, f0), spread_in(vs, b, f1)
            if mlp and mlp_aligned:
                lo = jnp.minimum(mlp_lo(tg, tc), F // MR - MPS)
                m3, m4 = mlp_descs(0, lo, MPS, sem, cond=c_mlp), mlp_descs(1, lo, MPS, sem, cond=c_mlp)
                if swap_m:
                    m3, m4 = mlp_descs(1, lo, MPS, sem, cond=c_mlp, prio=0), mlp_descs(0, lo, MPS, sem, cond=c_mlp, prio=1)
                n = min(len(p0), len(p1))
                for k in range(MPS - 1, -1, -1):
                    pos = (2 * k + 1) * n // (2 * MPS) + moff if mpos is None else int(mpos[k] * n)
                    p0.insert(pos, m3[k]); p1.insert(pos, m4[k])
            return interleave(p0, p1)

        PS = 3
        with scope('pro'):
            xcp = pltpu.make_async_copy(x_hbm, xbuf, sems.at[PS])
            xcp.start()
            if pro_spread:
                nq = QR // 8
                nwo = NWO * 8 // wo_rows
                n0 = min(nq, (nq * wq_split + nwo + 1) // 2 // wq_split)
                e0 = wq_descs(0, 0, n0, PS, prio=lambda i: 0) + mlp_descs(0, 0, MPRE, PS)
                e1 = wq_descs(0, n0, nq, PS, prio=lambda i: 1) + mlp_descs(1, 0, MPRE, PS)
                run(batch(0, 0, wq=False, extra0=e0, extra1=e1, phs=None if pph is None else (pph, pph)))
                run(batch(0, 1))
            else:
                run(wq_descs(0, 0, QR // 8, PS, prio=lambda i: i % 2))
                run(interleave(mlp_descs(0, 0, MPRE, PS), mlp_descs(1, 0, MPRE, PS)))
                for t in range(L):
                    run(batch(0, t, wq=(t > 0)))
        with scope('xwait'):
            xcp.wait()
            wait(wqbuf.at[0], PS)
            wait(mview(w3buf, 0, MPRE), PS)
            wait(mview(w4buf, 0, MPRE), PS)
        x = xbuf[...].astype(f32)
        xn = _layernorm(x).astype(bf16).astype(f32)
        xn8 = jnp.broadcast_to(xn, (8, D)).astype(bf16)
        row = jax.lax.broadcasted_iota(jnp.int32, (8, DH), 0)

        def womm(h, orow, sacc):
            lhs = jnp.broadcast_to(orow, (8, DH)).astype(bf16)
            a, i = h // HPQ, h % HPQ
            return sacc + jnp.dot(lhs, wobuf[a, i * DH:(i + 1) * DH, :], preferred_element_type=f32)

        def orow(h):
            return oall[h // NH, (h % NH):(h % NH) + 1, :]

        def group(g, last):
            m = jnp.full((8, 1), -jnp.inf, f32)
            l = jnp.zeros((8, 1), f32)
            acc = jnp.zeros((8, DH), f32)
            sacc = jnp.zeros((8, D), f32)
            qm = None
            for c in range(NC):
                tc = (c + L) % NC
                dg = (c + L) // NC
                tg = g + dg

                def do_wait():
                    with scope('wait'):
                        if last and c == NC - 1:
                            wait(kview(g, c), 0)
                            return
                        wait(kview(g, c), c)
                        wait(vview(g, c), c)
                        if last:
                            if c == 0:
                                wait(wqview(g, NC - 1), c)
                            return
                        wait(woview(g + 1, c), c)
                        if c == 0:
                            pl.when(g > 0)(lambda: wait(wqview(g, NC - 1), c))
                        else:
                            wait(wqview(g + 1, c - 1), c)

                        @pl.when(g < MG)
                        def _():
                            lo = jnp.minimum(mlp_lo(g, c), F // MR - MPS)
                            wait(mview(w3buf, lo, MPS), c)
                            wait(mview(w4buf, lo, MPS), c)

                if last:
                    if c == 0:
                        with scope('issue'):
                            run(batch(g, tc, wq=False, wo=False, mlp=False, rows=RL if last_from <= 2 else ROWS))
                        do_wait()
                    elif c == 1:
                        do_wait()
                        with scope('issue'):
                            run(batch(g, tc, wq=False, wo=False, mlp=False, ksem=0, rows=RL))
                            run([copy(wo_hbm.at[pl.ds(2, 2), pl.ds(i * x1rows, x1rows), :],
                                      wobuf.at[pl.ds(2, 2), pl.ds(i * x1rows, x1rows), :], 1, 1) for i in range(DH // x1rows)])
                    elif c == 2:
                        do_wait()
                        with scope('issue'):
                            run([copy(wo_hbm.at[1, pl.ds(i * 32, 32), :], wobuf.at[1, pl.ds(i * 32, 32), :], 2, 1)
                                 for i in range(DH // 32)])
                    else:
                        do_wait()
                        with scope('issue'):
                            run([copy(wo_hbm.at[0, pl.ds(i * 32, 32), :], wobuf.at[0, pl.ds(i * 32, 32), :], 0, 1)
                                 for i in range(R3 // 32)])
                else:
                    with scope('issue'):
                        if dg == 0:
                            run(batch(tg, tc, c_mlp=tg < MG))
                        else:
                            ok = tg < NG - 1
                            run(batch(tg, tc, c_wo=ok, c_wq=None if tc == 0 else ok, c_mlp=tg < MG))
                    do_wait()

                if c == 0 and do_compute:
                    wqg = wqbuf[g].reshape(D, GW)
                    q = jnp.dot(xn8, wqg, preferred_element_type=f32)
                    qm = [jnp.where(row == j, q[:, j * DH:(j + 1) * DH], 0.0).astype(bf16) for j in range(NH)]
                if do_compute:
                    s = None
                    for j in range(NH):
                        kj = kbuf[g * NH + j, pl.ds(c * CH, CH), :]
                        sj = jax.lax.dot_general(qm[j], kj, (((1,), (1,)), ((), ())), preferred_element_type=f32)
                        s = sj if s is None else s + sj
                    s = s * (DH ** -0.5)
                    m_new = jnp.maximum(m, jnp.max(s, axis=-1, keepdims=True))
                    alpha = jnp.exp(m - m_new)
                    p = jnp.exp(s - m_new)
                    l = l * alpha + jnp.sum(p, axis=-1, keepdims=True)
                    m = m_new
                    pb = p.astype(bf16)
                if last and c == NC - 1:
                    with scope('waitv'):
                        wait(vview(g, c), c)
                    run([copy(wo_hbm.at[0, pl.ds(i * 32, 32), :], wobuf.at[0, pl.ds(i * 32, 32), :], 3, 1)
                         for i in range(R3 // 32, DH // 32)])
                if do_compute:
                    pv = jnp.zeros((8, DH), f32)
                    for j in range(NH):
                        vj = vbuf[g * NH + j, pl.ds(c * CH, CH), :]
                        pv = pv + jnp.where(row == j, jnp.dot(pb, vj, preferred_element_type=f32), 0.0)
                    acc = acc * alpha + pv
                if last and c in early_steps and do_compute:
                    with scope('womm_early'):
                        heads = [h for h in range(H - NH) if h % HPQ != 0]
                        n = len(heads) // len(early_steps)
                        k = early_steps.index(c)
                        for h in heads[k * n:(k + 1) * n]:
                            sacc = womm(h, orow(h), sacc)
                        if k == 0:
                            ocol[0] = jnp.transpose(jnp.broadcast_to(orow(0), (DH, DH)))
                            ocol[1] = jnp.transpose(jnp.broadcast_to(orow(HPQ), (DH, DH)))
                if not last:
                    if c == 1:
                        @pl.when(g == mlp_comp)
                        def _():
                            with scope('mlp1'):
                                y = _layernorm(xn)
                                y8 = jnp.broadcast_to(y, (8, D)).astype(bf16)
                                hid = jax.lax.dot_general(y8, w3buf[...], (((1,), (1,)), ((), ())), preferred_element_type=f32)
                                hidbuf[...] = jax.nn.gelu(hid, approximate=True).astype(bf16)
                    if c == 2:
                        @pl.when(g == mlp_comp)
                        def _():
                            with scope('mlp2'):
                                h2 = jnp.dot(hidbuf[...], w4buf[...], preferred_element_type=f32)
                                b = xn + h2[0:1]
                                gatebuf[...] = b * jax.nn.sigmoid(b)
            o = acc / l if do_compute else acc
            if not last:
                oall[g] = o
                return None
            if do_compute:
                with scope('womm_last'):
                    for j in range(NH):
                        sacc = womm(g * NH + j, o[j:j + 1, :], sacc)
            def vpu_part(a, lo, hi):
                w0 = wobuf[a, lo:hi, :].astype(f32)
                oc = ocol[a, lo:hi, :]
                return jnp.concatenate([jnp.sum(w0[:, n * DH:(n + 1) * DH] * oc, axis=0, keepdims=True)
                                        for n in range(D // DH)], axis=1)

            with scope('waitX1'):
                wait(wobuf.at[pl.ds(2, 2), pl.ds(0, DH), :], 1)
            if do_compute:
                with scope('wommX1'):
                    for h in (2 * HPQ, 3 * HPQ):
                        sacc = womm(h, orow(h), sacc)
            s_row = sacc[0:1, :]
            gate = gatebuf[...]
            with scope('waitX2'):
                wait(wobuf.at[1, pl.ds(0, DH), :], 2)
            if do_compute:
                with scope('X2'):
                    s_row = s_row + vpu_part(1, 0, DH)
            with scope('waitX3a'):
                wait(wobuf.at[0, pl.ds(0, R3), :], 0)
            if do_compute:
                with scope('X3a'):
                    s_row = s_row + vpu_part(0, 0, R3)
            with scope('waitX3b'):
                wait(wobuf.at[0, pl.ds(R3, DH - R3), :], 3)
            if do_compute:
                with scope('X3b'):
                    s_row = s_row + vpu_part(0, R3, DH)
            with scope('final'):
                o_ref[...] = (x + s_row * gate).astype(o_ref.dtype)
            return None

        def body(g, _):
            group(g, False)
            return 0
        jax.lax.fori_loop(0, NG - 1, body, 0)
        group(NG - 1, True)

    def fn(A_x, A_k_cache, A_v_cache, A_wq, A_wo, B_x, B_w1, B_w2, B_w3, B_w4):
        B, Sq, D = A_x.shape
        _, H, Sk, DH = A_k_cache.shape
        W = min(4096, max(256, Sk // 4))
        F = B_w3.shape[1]
        NG = H // NH
        GW = NH * DH
        bf16 = jnp.bfloat16
        anyspec = pl.BlockSpec(memory_space=pl.ANY)
        out = pl.pallas_call(
            kernel,
            in_specs=[anyspec] * 7,
            out_specs=pl.BlockSpec(memory_space=pltpu.VMEM),
            out_shape=jax.ShapeDtypeStruct((1, D), A_x.dtype),
            scratch_shapes=[
                pltpu.VMEM((1, D), bf16),
                pltpu.VMEM((H, W, DH), bf16),
                pltpu.VMEM((H, W, DH), bf16),
                pltpu.VMEM((NG, QA, D // QA, GW), bf16),
                pltpu.VMEM((4, H * DH // 4, D), bf16),
                pltpu.VMEM((F, D), bf16),
                pltpu.VMEM((F, D), bf16),
                pltpu.VMEM((8, F), bf16),
                pltpu.VMEM((1, D), jnp.float32),
                pltpu.VMEM((NG, 8, DH), jnp.float32),
                pltpu.VMEM((2, DH, DH), jnp.float32),
                pltpu.SemaphoreType.DMA((R,)),
            ],
            compiler_params=pltpu.CompilerParams(
                vmem_limit_bytes=100 * 1024 * 1024,
                disable_bounds_checks=not bounds,
            ),
            interpret=interpret,
        )(A_x.reshape(1, D), A_k_cache, A_v_cache, A_wq.reshape(QA, D // QA, H * DH), A_wo.reshape(4, H * DH // 4, D), B_w3.T, B_w4)
        return out.reshape(B, Sq, D)
    return fn


_impl = build()


@jax.jit
def pallas_recurrent_scan__sliding_block_cached__mixer_s_mlp__decode_kernel(
    A_x: jax.Array,
    A_k_cache: jax.Array,
    A_v_cache: jax.Array,
    A_wq: jax.Array,
    A_wo: jax.Array,
    B_x: jax.Array,
    B_w1: jax.Array,
    B_w2: jax.Array,
    B_w3: jax.Array,
    B_w4: jax.Array,
):
    return _impl(A_x, A_k_cache, A_v_cache, A_wq, A_wo, B_x, B_w1, B_w2, B_w3, B_w4)
```

```python
import jax
import jax.numpy as jnp
import jax.experimental.pallas as pl
import jax.experimental.pallas.tpu as pltpu

NH = 4
NC = 4
LOOK = 2
ROWS = 24
NQ = 4
MR = 32
MPS = 2
MG = 5
MLP_G = 5
TAIL_SPLIT = 96


def _layernorm(x, eps=1e-5):
    m = jnp.mean(x, axis=-1, keepdims=True)
    xc = x - m
    v = jnp.mean(xc * xc, axis=-1, keepdims=True)
    return xc / jnp.sqrt(v + eps)


def _interleave(a, b):
    out = []
    for i in range(max(len(a), len(b))):
        out += a[i:i + 1] + b[i:i + 1]
    return out


def _spread(main, extra):
    pos = [int((i + 0.5) * len(main) / len(extra)) for i in range(len(extra))]
    out = []
    for i in range(len(main) + 1):
        out += [e for p, e in zip(pos, extra) if p == i] + main[i:i + 1]
    return out


def _kernel(x_hbm, k_hbm, v_hbm, wq_hbm, wo_hbm, w3_hbm, w4_hbm, o_ref,
            xbuf, kbuf, vbuf, wqbuf, wobuf, w3buf, w4buf, hidbuf, gatebuf, oall, ocol, sems):
    H, W, DH = kbuf.shape
    D = xbuf.shape[1]
    F = w3buf.shape[0]
    base = k_hbm.shape[2] - W
    NG = H // NH
    CH = W // NC
    GW = NH * DH
    QR = wq_hbm.shape[1]
    HPQ = H // NQ
    NWQ = QR // 8 // NC
    NWO = DH // 8 // NC
    NM = F // MR
    MPRE = NM - MG * NC * MPS
    f32, bf16 = jnp.float32, jnp.bfloat16

    def copy(src, dst, sem, prio, cond=None):
        def start():
            pltpu.make_async_copy(src, dst, sems.at[sem]).start(priority=prio)
        return start if cond is None else (lambda: pl.when(cond)(start))

    rb = [min(-(-CH * c // ROWS) * ROWS, W) for c in range(NC + 1)]

    def kv_descs(hbm, buf, g, c, sem, prio):
        return [copy(hbm.at[0, pl.ds(g * NH, NH), pl.ds(base + r, min(ROWS, rb[c + 1] - r)), :],
                     buf.at[pl.ds(g * NH, NH), pl.ds(r, min(ROWS, rb[c + 1] - r)), :], sem, prio)
                for r in range(rb[c], rb[c + 1], ROWS)]

    def wq_descs(g, lo, hi, sem, prio, cond=None):
        cols = pl.ds(pl.multiple_of(g * GW, GW), GW)
        return [copy(wq_hbm.at[:, pl.ds(i * 8, 8), cols], wqbuf.at[g, :, pl.ds(i * 8, 8), :], sem, prio, cond)
                for i in range(lo, hi)]

    def wo_descs(b, lo, hi, sem, cond=None):
        rows = [pl.ds(pl.multiple_of(b * DH + i * 8, 8), 8) for i in range(lo, hi)]
        return [copy(wo_hbm.at[:, r, :], wobuf.at[:, r, :], sem, 1, cond) for r in rows]

    def mlp_descs(which, lo, n, sem, cond=None):
        src, dst = ((w3_hbm, w3buf), (w4_hbm, w4buf))[which]
        rows = [pl.ds(pl.multiple_of((lo + k) * MR, MR), MR) for k in range(n)]
        return [copy(src.at[r, :], dst.at[r, :], sem, which, cond) for r in rows]

    def wo_head_descs(a, lo, hi, sem):
        return [copy(wo_hbm.at[a, pl.ds(r, 32), :], wobuf.at[a, pl.ds(r, 32), :], sem, 1) for r in range(lo, hi, 32)]

    def run(descs):
        for start in descs:
            start()

    def wait(view, sem):
        pltpu.make_async_copy(view, view, sems.at[sem]).wait()

    def kview(g, c): return kbuf.at[pl.ds(g * NH, NH), pl.ds(rb[c], rb[c + 1] - rb[c]), :]
    def vview(g, c): return vbuf.at[pl.ds(g * NH, NH), pl.ds(rb[c], rb[c + 1] - rb[c]), :]
    def wqview(g, p): return wqbuf.at[g, :, pl.ds(p * NWQ * 8, NWQ * 8), :]
    def woview(b, p): return wobuf.at[:, pl.ds(b * DH + p * NWO * 8, NWO * 8), :]
    def mview(buf, lo, n): return buf.at[pl.ds(lo * MR, n * MR), :]

    def mlp_lo(g, c):
        return jnp.minimum(MPRE + (g * NC + c) * MPS, NM - MPS)

    def batch(tg, tc, wq=True, wo=True, mlp=True, c_wq=None, c_wo=None, c_mlp=None, ksem=None,
              extra0=(), extra1=()):
        p0 = kv_descs(k_hbm, kbuf, tg, tc, tc if ksem is None else ksem, 0)
        p1 = kv_descs(v_hbm, vbuf, tg, tc, tc, 1)
        a, b = list(extra0), list(extra1)
        if wq:
            gq, pq = (tg, NC - 1) if tc == 0 else (tg + 1, tc - 1)
            if c_wq is not None:
                gq = jnp.minimum(gq, NG - 1)
            a = wq_descs(gq, pq * NWQ, (pq + 1) * NWQ, tc, 0, c_wq) + a
        if wo:
            bo = tg + 1 if c_wo is None else jnp.minimum(tg + 1, HPQ - 1)
            b = wo_descs(bo, tc * NWO, (tc + 1) * NWO, tc, c_wo) + b
        if a:
            p0, p1 = _spread(p0, a), _spread(p1, b)
        if mlp:
            lo = mlp_lo(tg, tc)
            m3, m4 = mlp_descs(0, lo, MPS, tc, c_mlp), mlp_descs(1, lo, MPS, tc, c_mlp)
            n = min(len(p0), len(p1))
            for k in reversed(range(MPS)):
                pos = (2 * k + 1) * n // (2 * MPS) + 5
                p0.insert(pos, m3[k])
                p1.insert(pos, m4[k])
        return _interleave(p0, p1)

    PS = NC - 1
    xcp = pltpu.make_async_copy(x_hbm, xbuf, sems.at[PS])
    xcp.start()
    nq = QR // 8
    n0 = (nq + NWO + 1) // 2
    run(batch(0, 0, wq=False,
              extra0=wq_descs(0, 0, n0, PS, 0) + mlp_descs(0, 0, MPRE, PS),
              extra1=wq_descs(0, n0, nq, PS, 1) + mlp_descs(1, 0, MPRE, PS)))
    run(batch(0, 1))
    xcp.wait()
    wait(wqbuf.at[0], PS)
    wait(mview(w3buf, 0, MPRE), PS)
    wait(mview(w4buf, 0, MPRE), PS)

    x = xbuf[...].astype(f32)
    xn = _layernorm(x).astype(bf16).astype(f32)
    xn8 = jnp.broadcast_to(xn, (8, D)).astype(bf16)
    row = jax.lax.broadcasted_iota(jnp.int32, (8, DH), 0)

    def womm(h, orow, sacc):
        lhs = jnp.broadcast_to(orow, (8, DH)).astype(bf16)
        a, i = h // HPQ, h % HPQ
        return sacc + jnp.dot(lhs, wobuf[a, i * DH:(i + 1) * DH, :], preferred_element_type=f32)

    def orow(h):
        return oall[h // NH, (h % NH):(h % NH) + 1, :]

    def group(g, last):
        m = jnp.full((8, 1), -jnp.inf, f32)
        l = jnp.zeros((8, 1), f32)
        acc = jnp.zeros((8, DH), f32)
        sacc = jnp.zeros((8, D), f32)
        qm = None
        for c in range(NC):
            tc, dg = (c + LOOK) % NC, (c + LOOK) // NC
            tg = g + dg if dg else g

            def wait_step():
                if last and c == NC - 1:
                    wait(kview(g, c), 0)
                    return
                wait(kview(g, c), c)
                wait(vview(g, c), c)
                if last:
                    if c == 0:
                        wait(wqview(g, NC - 1), c)
                    return
                wait(woview(g + 1, c), c)
                if c == 0:
                    pl.when(g > 0)(lambda: wait(wqview(g, NC - 1), c))
                else:
                    wait(wqview(g + 1, c - 1), c)

                @pl.when(g < MG)
                def _():
                    wait(mview(w3buf, mlp_lo(g, c), MPS), c)
                    wait(mview(w4buf, mlp_lo(g, c), MPS), c)

            if not last:
                if dg == 0:
                    run(batch(tg, tc, c_mlp=tg < MG))
                else:
                    more = tg < NG - 1
                    run(batch(tg, tc, c_wo=more, c_wq=None if tc == 0 else more, c_mlp=tg < MG))
                wait_step()
            elif c == 0:
                run(batch(g, tc, wq=False, wo=False, mlp=False))
                wait_step()
            else:
                wait_step()
                if c == 1:
                    run(batch(g, tc, wq=False, wo=False, mlp=False, ksem=0))
                    run([copy(wo_hbm.at[pl.ds(2, 2), pl.ds(r, 16), :], wobuf.at[pl.ds(2, 2), pl.ds(r, 16), :], 1, 1)
                         for r in range(0, DH, 16)])
                elif c == 2:
                    run(wo_head_descs(1, 0, DH, 2))
                else:
                    run(wo_head_descs(0, 0, TAIL_SPLIT, 0))

            if c == 0:
                q = jnp.dot(xn8, wqbuf[g].reshape(D, GW), preferred_element_type=f32)
                qm = [jnp.where(row == j, q[:, j * DH:(j + 1) * DH], 0.0).astype(bf16) for j in range(NH)]
            s = None
            for j in range(NH):
                kj = kbuf[g * NH + j, pl.ds(c * CH, CH), :]
                sj = jax.lax.dot_general(qm[j], kj, (((1,), (1,)), ((), ())), preferred_element_type=f32)
                s = sj if s is None else s + sj
            s = s * (DH ** -0.5)
            m_new = jnp.maximum(m, jnp.max(s, axis=-1, keepdims=True))
            alpha = jnp.exp(m - m_new)
            p = jnp.exp(s - m_new)
            l = l * alpha + jnp.sum(p, axis=-1, keepdims=True)
            m = m_new
            pb = p.astype(bf16)
            if last and c == NC - 1:
                wait(vview(g, c), c)
                run(wo_head_descs(0, TAIL_SPLIT, DH, 3))
            pv = jnp.zeros((8, DH), f32)
            for j in range(NH):
                vj = vbuf[g * NH + j, pl.ds(c * CH, CH), :]
                pv = pv + jnp.where(row == j, jnp.dot(pb, vj, preferred_element_type=f32), 0.0)
            acc = acc * alpha + pv

            if last and c == 0:
                for h in range(H - NH):
                    if h % HPQ != 0:
                        sacc = womm(h, orow(h), sacc)
                for a in range(2):
                    ocol[a] = jnp.transpose(jnp.broadcast_to(orow(a * HPQ), (DH, DH)))
            if not last and c == 1:
                @pl.when(g == MLP_G)
                def _():
                    y8 = jnp.broadcast_to(_layernorm(xn), (8, D)).astype(bf16)
                    hid = jax.lax.dot_general(y8, w3buf[...], (((1,), (1,)), ((), ())), preferred_element_type=f32)
                    hidbuf[...] = jax.nn.gelu(hid, approximate=True).astype(bf16)
            if not last and c == 2:
                @pl.when(g == MLP_G)
                def _():
                    b = xn + jnp.dot(hidbuf[...], w4buf[...], preferred_element_type=f32)[0:1]
                    gatebuf[...] = b * jax.nn.sigmoid(b)

        o = acc / l
        if not last:
            oall[g] = o
            return

        def vpu_part(a, lo, hi):
            w = wobuf[a, lo:hi, :].astype(f32)
            oc = ocol[a, lo:hi, :]
            return jnp.concatenate([jnp.sum(w[:, n * DH:(n + 1) * DH] * oc, axis=0, keepdims=True)
                                    for n in range(D // DH)], axis=1)

        for j in range(NH):
            sacc = womm(g * NH + j, o[j:j + 1, :], sacc)
        wait(wobuf.at[pl.ds(2, 2), pl.ds(0, DH), :], 1)
        for h in (2 * HPQ, 3 * HPQ):
            sacc = womm(h, orow(h), sacc)
        s_row = sacc[0:1, :]
        gate = gatebuf[...]
        wait(wobuf.at[1, pl.ds(0, DH), :], 2)
        s_row = s_row + vpu_part(1, 0, DH)
        wait(wobuf.at[0, pl.ds(0, TAIL_SPLIT), :], 0)
        s_row = s_row + vpu_part(0, 0, TAIL_SPLIT)
        wait(wobuf.at[0, pl.ds(TAIL_SPLIT, DH - TAIL_SPLIT), :], 3)
        s_row = s_row + vpu_part(0, TAIL_SPLIT, DH)
        o_ref[...] = (x + s_row * gate).astype(o_ref.dtype)

    def body(g, carry):
        group(g, False)
        return carry

    jax.lax.fori_loop(0, NG - 1, body, 0)
    group(NG - 1, True)


@jax.jit
def pallas_recurrent_scan__sliding_block_cached__mixer_s_mlp__decode_kernel(
    A_x: jax.Array,
    A_k_cache: jax.Array,
    A_v_cache: jax.Array,
    A_wq: jax.Array,
    A_wo: jax.Array,
    B_x: jax.Array,
    B_w1: jax.Array,
    B_w2: jax.Array,
    B_w3: jax.Array,
    B_w4: jax.Array,
):
    B, Sq, D = A_x.shape
    _, H, Sk, DH = A_k_cache.shape
    W = min(4096, max(256, Sk // 4))
    F = B_w3.shape[1]
    NG = H // NH
    bf16, f32 = jnp.bfloat16, jnp.float32
    hbm = pl.BlockSpec(memory_space=pl.ANY)
    out = pl.pallas_call(
        _kernel,
        in_specs=[hbm] * 7,
        out_specs=pl.BlockSpec(memory_space=pltpu.VMEM),
        out_shape=jax.ShapeDtypeStruct((1, D), A_x.dtype),
        scratch_shapes=[
            pltpu.VMEM((1, D), bf16),
            pltpu.VMEM((H, W, DH), bf16),
            pltpu.VMEM((H, W, DH), bf16),
            pltpu.VMEM((NG, NQ, D // NQ, NH * DH), bf16),
            pltpu.VMEM((NQ, H * DH // NQ, D), bf16),
            pltpu.VMEM((F, D), bf16),
            pltpu.VMEM((F, D), bf16),
            pltpu.VMEM((8, F), bf16),
            pltpu.VMEM((1, D), f32),
            pltpu.VMEM((NG, 8, DH), f32),
            pltpu.VMEM((2, DH, DH), f32),
            pltpu.SemaphoreType.DMA((NC,)),
        ],
        compiler_params=pltpu.CompilerParams(
            vmem_limit_bytes=100 * 1024 * 1024,
            disable_bounds_checks=True,
        ),
    )(
        A_x.reshape(1, D),
        A_k_cache,
        A_v_cache,
        A_wq.reshape(NQ, D // NQ, H * DH),
        A_wo.reshape(NQ, H * DH // NQ, D),
        B_w3.T,
        B_w4,
    )
    return out.reshape(B, Sq, D)
```

```python
import jax
import jax.numpy as jnp
import jax.experimental.pallas as pl
import jax.experimental.pallas.tpu as pltpu

NH = 4
NC = 4
LOOK = 2
ROWS = (32, 16)
NQ = 4
MR = 32
MPS = 2
MG = 5
MLP_G = 5
TAIL_SPLIT = 96


def _layernorm(x, eps=1e-5):
    m = jnp.mean(x, axis=-1, keepdims=True)
    xc = x - m
    v = jnp.mean(xc * xc, axis=-1, keepdims=True)
    return xc / jnp.sqrt(v + eps)


def _interleave(a, b):
    out = []
    for i in range(max(len(a), len(b))):
        out += a[i:i + 1] + b[i:i + 1]
    return out


def _spread(main, extra):
    pos = [int((i + 0.5) * len(main) / len(extra)) for i in range(len(extra))]
    out = []
    for i in range(len(main) + 1):
        out += [e for p, e in zip(pos, extra) if p == i] + main[i:i + 1]
    return out


def _kernel(*refs):
    pl.run_scoped(lambda sems: _body(*refs, sems), pltpu.SemaphoreType.DMA((NC,)))


def _body(x_hbm, k_hbm, v_hbm, wq_hbm, wo_hbm, w3_hbm, w4_hbm, o_ref,
          xbuf, kbuf, vbuf, wqbuf, wobuf, w3buf, w4buf, hidbuf, gatebuf, oall, ocol, sems):
    H, W, DH = kbuf.shape
    D = xbuf.shape[1]
    F = w3buf.shape[0]
    base = k_hbm.shape[2] - W
    NG = H // NH
    CH = W // NC
    GW = NH * DH
    QR = wq_hbm.shape[1]
    HPQ = H // NQ
    NWQ = QR // 8 // NC
    NWO = DH // 8 // NC
    NM = F // MR
    MPRE = NM - MG * NC * MPS
    f32, bf16 = jnp.float32, jnp.bfloat16

    def copy(src, dst, sem, prio, cond=None):
        def start():
            pltpu.make_async_copy(src, dst, sems.at[sem]).start(priority=prio)
        return start if cond is None else (lambda: pl.when(cond)(start))

    cuts = [0]
    while cuts[-1] < W:
        cuts.append(min(W, cuts[-1] + ROWS[(len(cuts) - 1) % len(ROWS)]))
    rb = [min(r for r in cuts if r >= CH * c) for c in range(NC + 1)]

    def kv_descs(hbm, buf, g, c, sem, prio):
        return [copy(hbm.at[0, pl.ds(g * NH, NH), pl.ds(base + lo, hi - lo), :],
                     buf.at[pl.ds(g * NH, NH), pl.ds(lo, hi - lo), :], sem, prio)
                for lo, hi in zip(cuts[:-1], cuts[1:]) if rb[c] <= lo < rb[c + 1]]

    def wq_descs(g, lo, hi, sem, prio, cond=None):
        cols = pl.ds(pl.multiple_of(g * GW, GW), GW)
        return [copy(wq_hbm.at[:, pl.ds(i * 8, 8), cols], wqbuf.at[g, :, pl.ds(i * 8, 8), :], sem, prio, cond)
                for i in range(lo, hi)]

    def wo_descs(b, lo, hi, sem, cond=None):
        rows = [pl.ds(pl.multiple_of(b * DH + i * 8, 8), 8) for i in range(lo, hi)]
        return [copy(wo_hbm.at[:, r, :], wobuf.at[:, r, :], sem, 1, cond) for r in rows]

    def mlp_descs(which, lo, n, sem, cond=None):
        src, dst = ((w3_hbm, w3buf), (w4_hbm, w4buf))[which]
        rows = [pl.ds(pl.multiple_of((lo + k) * MR, MR), MR) for k in range(n)]
        return [copy(src.at[r, :], dst.at[r, :], sem, which, cond) for r in rows]

    def wo_head_descs(a, lo, hi, sem):
        return [copy(wo_hbm.at[a, pl.ds(r, 32), :], wobuf.at[a, pl.ds(r, 32), :], sem, 1) for r in range(lo, hi, 32)]

    def run(descs):
        for start in descs:
            start()

    def wait(view, sem):
        pltpu.make_async_copy(view, view, sems.at[sem]).wait()

    def kview(g, c): return kbuf.at[pl.ds(g * NH, NH), pl.ds(rb[c], rb[c + 1] - rb[c]), :]
    def vview(g, c): return vbuf.at[pl.ds(g * NH, NH), pl.ds(rb[c], rb[c + 1] - rb[c]), :]
    def wqview(g, p): return wqbuf.at[g, :, pl.ds(p * NWQ * 8, NWQ * 8), :]
    def woview(b, p): return wobuf.at[:, pl.ds(b * DH + p * NWO * 8, NWO * 8), :]
    def mview(buf, lo, n): return buf.at[pl.ds(lo * MR, n * MR), :]

    def mlp_lo(g, c):
        return jnp.minimum(MPRE + (g * NC + c) * MPS, NM - MPS)

    def batch(tg, tc, wq=True, wo=True, mlp=True, c_wq=None, c_wo=None, c_mlp=None, ksem=None,
              extra0=(), extra1=()):
        p0 = kv_descs(k_hbm, kbuf, tg, tc, tc if ksem is None else ksem, 0)
        p1 = kv_descs(v_hbm, vbuf, tg, tc, tc, 1)
        a, b = list(extra0), list(extra1)
        if wq:
            gq, pq = (tg, NC - 1) if tc == 0 else (tg + 1, tc - 1)
            if c_wq is not None:
                gq = jnp.minimum(gq, NG - 1)
            a = wq_descs(gq, pq * NWQ, (pq + 1) * NWQ, tc, 0, c_wq) + a
        if wo:
            bo = tg + 1 if c_wo is None else jnp.minimum(tg + 1, HPQ - 1)
            b = wo_descs(bo, tc * NWO, (tc + 1) * NWO, tc, c_wo) + b
        if a:
            p0, p1 = _spread(p0, a), _spread(p1, b)
        if mlp:
            lo = mlp_lo(tg, tc)
            m3, m4 = mlp_descs(0, lo, MPS, tc, c_mlp), mlp_descs(1, lo, MPS, tc, c_mlp)
            n = min(len(p0), len(p1))
            for k in reversed(range(MPS)):
                pos = (2 * k + 1) * n // (2 * MPS) + 5
                p0.insert(pos, m3[k])
                p1.insert(pos, m4[k])
        return _interleave(p0, p1)

    PS = NC - 1
    xcp = pltpu.make_async_copy(x_hbm, xbuf, sems.at[PS])
    xcp.start()
    nq = QR // 8
    n0 = (nq + NWO + 1) // 2
    run(batch(0, 0, wq=False,
              extra0=wq_descs(0, 0, n0, PS, 0) + mlp_descs(0, 0, MPRE, PS),
              extra1=wq_descs(0, n0, nq, PS, 1) + mlp_descs(1, 0, MPRE, PS)))
    run(batch(0, 1))
    xcp.wait()
    wait(wqbuf.at[0], PS)
    wait(mview(w3buf, 0, MPRE), PS)
    wait(mview(w4buf, 0, MPRE), PS)

    x = xbuf[...].astype(f32)
    xn = _layernorm(x).astype(bf16).astype(f32)
    xn8 = jnp.broadcast_to(xn, (8, D)).astype(bf16)
    row = jax.lax.broadcasted_iota(jnp.int32, (8, DH), 0)

    def womm(h, orow, sacc):
        lhs = jnp.broadcast_to(orow, (8, DH)).astype(bf16)
        a, i = h // HPQ, h % HPQ
        return sacc + jnp.dot(lhs, wobuf[a, i * DH:(i + 1) * DH, :], preferred_element_type=f32)

    def orow(h):
        return oall[h // NH, (h % NH):(h % NH) + 1, :]

    def group(g, last):
        m = jnp.full((8, 1), -jnp.inf, f32)
        l = jnp.zeros((8, 1), f32)
        acc = jnp.zeros((8, DH), f32)
        sacc = jnp.zeros((8, D), f32)
        qm = None
        for c in range(NC):
            tc, dg = (c + LOOK) % NC, (c + LOOK) // NC
            tg = g + dg if dg else g

            def wait_step():
                if last and c == NC - 1:
                    wait(kview(g, c), 0)
                    return
                wait(kview(g, c), c)
                wait(vview(g, c), c)
                if last:
                    if c == 0:
                        wait(wqview(g, NC - 1), c)
                    return
                wait(woview(g + 1, c), c)
                if c == 0:
                    pl.when(g > 0)(lambda: wait(wqview(g, NC - 1), c))
                else:
                    wait(wqview(g + 1, c - 1), c)

                @pl.when(g < MG)
                def _():
                    wait(mview(w3buf, mlp_lo(g, c), MPS), c)
                    wait(mview(w4buf, mlp_lo(g, c), MPS), c)

            if not last:
                if dg == 0:
                    run(batch(tg, tc, c_mlp=tg < MG))
                else:
                    more = tg < NG - 1
                    run(batch(tg, tc, c_wo=more, c_wq=None if tc == 0 else more, c_mlp=tg < MG))
                wait_step()
            elif c == 0:
                run(batch(g, tc, wq=False, wo=False, mlp=False))
                wait_step()
            else:
                wait_step()
                if c == 1:
                    run(batch(g, tc, wq=False, wo=False, mlp=False, ksem=0))
                    run([copy(wo_hbm.at[pl.ds(2, 2), pl.ds(r, 16), :], wobuf.at[pl.ds(2, 2), pl.ds(r, 16), :], 1, 1)
                         for r in range(0, DH, 16)])
                elif c == 2:
                    run(wo_head_descs(1, 0, DH, 2))
                else:
                    run(wo_head_descs(0, 0, TAIL_SPLIT, 0))

            if c == 0:
                q = jnp.dot(xn8, wqbuf[g].reshape(D, GW), preferred_element_type=f32)
                qm = [jnp.where(row == j, q[:, j * DH:(j + 1) * DH], 0.0).astype(bf16) for j in range(NH)]
            s = None
            for j in range(NH):
                kj = kbuf[g * NH + j, pl.ds(c * CH, CH), :]
                sj = jax.lax.dot_general(qm[j], kj, (((1,), (1,)), ((), ())), preferred_element_type=f32)
                s = sj if s is None else s + sj
            s = s * (DH ** -0.5)
            m_new = jnp.maximum(m, jnp.max(s, axis=-1, keepdims=True))
            alpha = jnp.exp(m - m_new)
            p = jnp.exp(s - m_new)
            l = l * alpha + jnp.sum(p, axis=-1, keepdims=True)
            m = m_new
            pb = p.astype(bf16)
            if last and c == NC - 1:
                wait(vview(g, c), c)
                run(wo_head_descs(0, TAIL_SPLIT, DH, 3))
            pv = jnp.zeros((8, DH), f32)
            for j in range(NH):
                vj = vbuf[g * NH + j, pl.ds(c * CH, CH), :]
                pv = pv + jnp.where(row == j, jnp.dot(pb, vj, preferred_element_type=f32), 0.0)
            acc = acc * alpha + pv

            if last and c == 0:
                for h in range(H - NH):
                    if h % HPQ != 0:
                        sacc = womm(h, orow(h), sacc)
                for a in range(2):
                    ocol[a] = jnp.transpose(jnp.broadcast_to(orow(a * HPQ), (DH, DH)))
            if not last and c == 1:
                @pl.when(g == MLP_G)
                def _():
                    y8 = jnp.broadcast_to(_layernorm(xn), (8, D)).astype(bf16)
                    hid = jax.lax.dot_general(y8, w3buf[...], (((1,), (1,)), ((), ())), preferred_element_type=f32)
                    hidbuf[...] = jax.nn.gelu(hid, approximate=True).astype(bf16)
            if not last and c == 2:
                @pl.when(g == MLP_G)
                def _():
                    b = xn + jnp.dot(hidbuf[...], w4buf[...], preferred_element_type=f32)[0:1]
                    gatebuf[...] = b * jax.nn.sigmoid(b)

        o = acc / l
        if not last:
            oall[g] = o
            return

        def vpu_part(a, lo, hi):
            w = wobuf[a, lo:hi, :].astype(f32)
            oc = ocol[a, lo:hi, :]
            return jnp.concatenate([jnp.sum(w[:, n * DH:(n + 1) * DH] * oc, axis=0, keepdims=True)
                                    for n in range(D // DH)], axis=1)

        for j in range(NH):
            sacc = womm(g * NH + j, o[j:j + 1, :], sacc)
        wait(wobuf.at[pl.ds(2, 2), pl.ds(0, DH), :], 1)
        for h in (2 * HPQ, 3 * HPQ):
            sacc = womm(h, orow(h), sacc)
        s_row = sacc[0:1, :]
        gate = gatebuf[...]
        wait(wobuf.at[1, pl.ds(0, DH), :], 2)
        s_row = s_row + vpu_part(1, 0, DH)
        wait(wobuf.at[0, pl.ds(0, TAIL_SPLIT), :], 0)
        s_row = s_row + vpu_part(0, 0, TAIL_SPLIT)
        wait(wobuf.at[0, pl.ds(TAIL_SPLIT, DH - TAIL_SPLIT), :], 3)
        s_row = s_row + vpu_part(0, TAIL_SPLIT, DH)
        o_ref[...] = (x + s_row * gate).astype(o_ref.dtype)

    def body(g, carry):
        group(g, False)
        return carry

    jax.lax.fori_loop(0, NG - 1, body, 0)
    group(NG - 1, True)


@jax.jit
def pallas_recurrent_scan__sliding_block_cached__mixer_s_mlp__decode_kernel(
    A_x: jax.Array,
    A_k_cache: jax.Array,
    A_v_cache: jax.Array,
    A_wq: jax.Array,
    A_wo: jax.Array,
    B_x: jax.Array,
    B_w1: jax.Array,
    B_w2: jax.Array,
    B_w3: jax.Array,
    B_w4: jax.Array,
):
    B, Sq, D = A_x.shape
    _, H, Sk, DH = A_k_cache.shape
    W = min(4096, max(256, Sk // 4))
    F = B_w3.shape[1]
    NG = H // NH
    bf16, f32 = jnp.bfloat16, jnp.float32
    hbm = pl.BlockSpec(memory_space=pl.ANY)
    out = pl.pallas_call(
        _kernel,
        in_specs=[hbm] * 7,
        out_specs=pl.BlockSpec(memory_space=pltpu.VMEM),
        out_shape=jax.ShapeDtypeStruct((1, D), A_x.dtype),
        scratch_shapes=[
            pltpu.VMEM((1, D), bf16),
            pltpu.VMEM((H, W, DH), bf16),
            pltpu.VMEM((H, W, DH), bf16),
            pltpu.VMEM((NG, NQ, D // NQ, NH * DH), bf16),
            pltpu.VMEM((NQ, H * DH // NQ, D), bf16),
            pltpu.VMEM((F, D), bf16),
            pltpu.VMEM((F, D), bf16),
            pltpu.VMEM((8, F), bf16),
            pltpu.VMEM((1, D), f32),
            pltpu.VMEM((NG, 8, DH), f32),
            pltpu.VMEM((2, DH, DH), f32),
        ],
        compiler_params=pltpu.CompilerParams(
            vmem_limit_bytes=100 * 1024 * 1024,
            disable_bounds_checks=True,
        ),
    )(
        A_x.reshape(1, D),
        A_k_cache,
        A_v_cache,
        A_wq.reshape(NQ, D // NQ, H * DH),
        A_wo.reshape(NQ, H * DH // NQ, D),
        B_w3.T,
        B_w4,
    )
    return out.reshape(B, Sq, D)
```
